```python
import jax
import jax.numpy as jnp

def _softmax(x, axis=-1):
    return jax.nn.softmax(x, axis=axis)
def _gelu(x):
    return jax.nn.gelu(x, approximate=True)
def _silu(x):
    return jax.nn.silu(x)
def _sigmoid(x):
    return jax.nn.sigmoid(x)
def _layernorm(x, axis=-1, eps=1e-5):
    m = jnp.mean(x, axis=axis, keepdims=True)
    v = jnp.var(x, axis=axis, keepdims=True)
    return (x - m) / jnp.sqrt(v + eps)
def _scatter_add(tgt, idx, src, axis=0):
    return tgt.at[idx].add(src)
def _segment_sum(src, seg, n):
    return jax.ops.segment_sum(src, seg, n)
class _Rng:
    def __init__(self, key):
        self._k = key
    def _next(self):
        self._k, sub = jax.random.split(self._k)
        return sub
    def normal(self, shape):
        return jax.random.normal(self._next(), shape, dtype=jnp.bfloat16)
    def randint(self, lo, hi, shape):
        return jax.random.randint(self._next(), shape, lo, hi, dtype=jnp.int32)
    def uniform(self, shape, lo=0.0, hi=1.0):
        return jax.random.uniform(self._next(), shape, jnp.bfloat16, lo, hi)
    def permutation(self, n):
        return jax.random.permutation(self._next(), n)


kernel_name = 'parallel_sum__sliding_local_dilated__glu_gated_geglu__prompt'

def setup_inputs():
    _rng = _Rng(jax.random.key(int.from_bytes(__import__("os").urandom(4), "little")))
    _w = (lambda a: (lambda t: t.astype(jnp.bfloat16) if jnp.issubdtype(t.dtype, jnp.floating) else t)(jnp.asarray(a)))
    def _A_setup():
        B, S, D = 1, 2048, 1024
        return {
            "x": _w((lambda *s: _rng.normal(s) * 0.05)(B, S, D)),
            "wqkv": _w((lambda *s: _rng.normal(s) * 0.05)(D, 3 * D)),
            "wo": _w((lambda *s: _rng.normal(s) * 0.05)(D, D)),
        }
    _A_in = _A_setup()

    def _B_setup():
        B, S, Dm, Df = 1, 2048, 1024, 3584
        return {
            "x": _w((lambda *s: _rng.normal(s) * 0.05)(B, S, Dm)),
            "w_gate": _w((lambda *s: _rng.normal(s) * 0.05)(Dm, Df) * (Dm ** -0.5)),
            "w_up": _w((lambda *s: _rng.normal(s) * 0.05)(Dm, Df) * (Dm ** -0.5)),
            "w_down": _w((lambda *s: _rng.normal(s) * 0.05)(Df, Dm) * (Df ** -0.5)),
        }
    _B_in = _B_setup()

    return {
        "A_x": _A_in["x"],
        "A_wqkv": _A_in["wqkv"],
        "A_wo": _A_in["wo"],
        "B_x": _B_in["x"],
        "B_w_gate": _B_in["w_gate"],
        "B_w_up": _B_in["w_up"],
        "B_w_down": _B_in["w_down"],
    }

def reference(A_x, A_wqkv, A_wo, B_x, B_w_gate, B_w_up, B_w_down):
    def _A_ref(x, wqkv, wo):
        B, S, D = x.shape
        H = 32; Dh = D // H
        W, dil = 8, 2
        qkv = (lambda x, *d: x.transpose(*d))((x @ wqkv).reshape(B, S, 3, H, Dh), 2, 0, 3, 1, 4)
        q, k, v = qkv[0], qkv[1], qkv[2]
        scale = Dh ** -0.5
        pos = jnp.arange(S)
        off = jnp.arange(W) * dil
        idx = pos[:, None] - off[None, :]
        mask = idx >= 0
        idx_c = jnp.where(mask, idx, 0).reshape(-1)
        kg = k[:, :, idx_c, :].reshape(B, H, S, W, Dh)
        vg = v[:, :, idx_c, :].reshape(B, H, S, W, Dh)
        logits = jnp.einsum("bhsd,bhswd->bhsw", q, kg) * scale
        logits = jnp.where(mask[None, None, :, :], logits, -1e9)
        attn = _softmax(logits, axis=-1)
        o = jnp.einsum("bhsw,bhswd->bhsd", attn, vg)
        return (lambda x, *d: x.transpose(*d))(o, 0, 2, 1, 3).reshape(B, S, D) @ wo

    def _B_ref(x, w_gate, w_up, w_down):
        g = jnp.einsum("bsd,df->bsf", x, w_gate)
        u = jnp.einsum("bsd,df->bsf", x, w_up)
        h = _gelu(g) * u
        return jnp.einsum("bsf,fd->bsd", h, w_down)

    x = A_x
    xn = _layernorm(x, axis=-1)
    return x + _A_ref(xn, A_wqkv, A_wo) + _B_ref(xn, B_w_gate, B_w_up, B_w_down)
```

```python
import functools
import numpy as np
import jax
import jax.numpy as jnp
from jax import lax
from jax.experimental import pallas as pl
from jax.experimental.pallas import tpu as pltpu

S, D, F = 2048, 1024, 3584
H, DH, W, DIL = 32, 32, 8, 2
HALO = 16
NC = D // 128
f32, bf16, u32 = jnp.float32, jnp.bfloat16, jnp.uint32


def _gelu(x):
    c = float(np.sqrt(2.0 / np.pi))
    return x * (0.5 * (1.0 + jnp.tanh(c * (x + 0.044715 * (x * x * x)))))


def build(TM=256, FA=256, FB=(256, 512), TF=512, lnchain=False, PR=64, qk_st=8, pv_st=8, pchain=False, WST=33, nobc=False):
    NB = S // TM
    TF0 = FA + sum(FB)
    FR = F - TF0
    NCH = FR // TF
    assert NCH * TF == FR
    KP = D // NB
    assert NB == NC

    def kern(x_hbm, wqkv_hbm, wo_hbm, wg_hbm, wu_hbm, wd_hbm, out_hbm,
             x_v, xn_v, acc_v, wqkv_r, wqkv_p, wo_r, wo_f, wo_p,
             wgu_a, wg0, wu0, wd0, wg1, wu1, wd1,
             h0_v, q_s, k_s, v_s, o_s, h_s, out_v, xsem, qsem, wosem, wsem, osem):

        def blk(i):
            return pl.ds(pl.multiple_of(i * TM, TM), TM)

        def x_copy(i):
            return pltpu.make_async_copy(x_hbm.at[blk(i)], x_v.at[blk(i)], xsem.at[i])

        def o_copy(i):
            return pltpu.make_async_copy(out_v.at[blk(i)], out_hbm.at[blk(i)], osem.at[i])

        def qkv_copy(i):
            rows = pl.ds(pl.multiple_of(i * KP, KP), KP)
            return pltpu.make_async_copy(wqkv_hbm.at[rows], wqkv_r.at[rows], qsem.at[i])

        def wo_copy(i):
            cols = pl.ds(pl.multiple_of(i * 128, 128), 128)
            return pltpu.make_async_copy(wo_hbm.at[:, cols], wo_r.at[i], wosem.at[i])

        a_copies = [
            pltpu.make_async_copy(wg_hbm.at[:, pl.ds(0, FA)], wgu_a.at[:, pl.ds(0, FA)], wsem.at[0]),
            pltpu.make_async_copy(wu_hbm.at[:, pl.ds(0, FA)], wgu_a.at[:, pl.ds(FA, FA)], wsem.at[1]),
        ]
        def b_piece(i):
            r = pl.ds(pl.multiple_of(i * KP, KP), KP)
            rd = pl.ds(pl.multiple_of(i * (TF0 // NB), TF0 // NB), TF0 // NB)
            return [
                pltpu.make_async_copy(wg_hbm.at[r, pl.ds(FA, TF0 - FA)], wg0.at[r], wsem.at[2]),
                pltpu.make_async_copy(wu_hbm.at[r, pl.ds(FA, TF0 - FA)], wu0.at[r], wsem.at[3]),
                pltpu.make_async_copy(wd_hbm.at[rd], wd0.at[rd], wsem.at[4]),
            ]

        b_copies = [
            pltpu.make_async_copy(wg0, wg0, wsem.at[2]),
            pltpu.make_async_copy(wu0, wu0, wsem.at[3]),
            pltpu.make_async_copy(wd0, wd0, wsem.at[4]),
        ]
        c_copies = [
            pltpu.make_async_copy(wg_hbm.at[:, pl.ds(TF0, FR)], wg1, wsem.at[5]),
            pltpu.make_async_copy(wu_hbm.at[:, pl.ds(TF0, FR)], wu1, wsem.at[6]),
            pltpu.make_async_copy(wd_hbm.at[pl.ds(TF0, FR), :], wd1, wsem.at[7]),
        ]
        x_copy(0).start()
        for c in a_copies:
            c.start()
        x_copy(1).start()

        def layernorm(i):
            prev = None
            step = 16 if lnchain else TM
            for r in range(0, TM, step):
                rows = pl.ds(pl.multiple_of(i * TM + r, 16), step)
                x = x_v[rows, :].astype(f32)
                if prev is not None:
                    x = jnp.where(i < 0, prev, x)
                m = jnp.mean(x, axis=-1, keepdims=True)
                xc = x - m
                var = jnp.mean(xc * xc, axis=-1, keepdims=True)
                prev = xc * lax.rsqrt(var + 1e-5)
                xn_v[rows, :] = prev.astype(bf16)

        def reorder_wqkv(i):
            shp = (PR // 2, 128)
            lane = lax.broadcasted_iota(jnp.int32, shp, 1)
            grp = (lane >> 2) & 7
            prev = None
            for r in range(0, KP, PR):
                rows = pl.ds(pl.multiple_of(i * KP + r, PR), PR)
                for part in range(3):
                    a = []
                    for cs in range(NC):
                        cd = (grp - cs) & 7
                        dl = ((lane >> 5) - (grp < cd).astype(jnp.int32)) & 3
                        idx = (lane & 3) * 32 + cd * 4 + dl
                        w = pltpu.bitcast(wqkv_r[rows, pl.ds(part * D + cs * 128, 128)], u32)
                        if pchain and prev is not None:
                            w = jnp.where(i < 0, prev, w)
                        a.append(jnp.take_along_axis(w, idx, axis=1))
                    a = [a[(-j) % 8] for j in range(8)]
                    for b in (1, 2, 4):
                        sel = (grp & b) != 0
                        a = [jnp.where(sel, a[(j - b) % 8], a[j]) for j in range(8)]
                    for cd in range(NC):
                        w = a[cd] if cd == 0 else pltpu.roll(a[cd], 128 - 4 * cd, 1)
                        wqkv_p[rows, pl.ds(part * D + cd * 128, 128)] = pltpu.bitcast(w, bf16)
                        prev = w

        def reorder_wo(i):
            cols = pl.ds(pl.multiple_of(i * 128, 128), 128)
            for h in range(H):
                wo_f[pl.ds(h * WST, DH), :] = wo_r[i, pl.ds(h * DH, DH), :].astype(f32)
            for d in range(DH):
                wo_p[pl.ds(d * H, H), cols] = wo_f[pl.ds(d, H, stride=WST), :].astype(bf16)

        for c in range(NC):
            k_s[c, pl.ds(TM, HALO), :] = jnp.zeros((HALO, 128), f32)
            v_s[c, pl.ds(TM, HALO), :] = jnp.zeros((HALO, 128), f32)

        x_copy(0).wait()
        layernorm(0)
        for c in a_copies:
            c.wait()

        def phase_a(i, carry):
            nxt = jnp.minimum(i + 1, NB - 1)
            pl.when(i + 2 < NB)(x_copy(jnp.minimum(i + 2, NB - 1)).start)
            for c in b_piece(i):
                c.start()

            @pl.when(i >= NB - 2)
            def _():
                qkv_copy(i - (NB - 2)).start()
                wo_copy(i - (NB - 2)).start()

            pl.when(i + 1 < NB)(x_copy(nxt).wait)
            rows = blk(i)
            gu = jnp.dot(xn_v[rows, :], wgu_a[...], preferred_element_type=f32)
            h0_v[rows, pl.ds(0, FA)] = (_gelu(gu[:, :FA]) * gu[:, FA:]).astype(bf16)
            layernorm(nxt)
            return carry

        lax.fori_loop(0, NB, phase_a, 0)
        for c in b_copies:
            c.wait()

        def phase_b(i, carry):
            @pl.when(i + 2 < NB)
            def _():
                qkv_copy(i + 2).start()
                wo_copy(i + 2).start()

            for j, c in enumerate(c_copies):
                pl.when(i == 2 * j)(c.start)
            qkv_copy(i).wait()
            wo_copy(i).wait()
            rows = blk(i)
            xn = xn_v[rows, :]
            off = 0
            for fb in FB:
                cols = pl.ds(off, fb)
                g = jnp.dot(xn, wg0[:, cols], preferred_element_type=f32)
                u = jnp.dot(xn, wu0[:, cols], preferred_element_type=f32)
                h0_v[rows, pl.ds(FA + off, fb)] = (_gelu(g) * u).astype(bf16)
                off += fb
            reorder_wqkv(i)
            reorder_wo(i)
            acc_v[rows, :] = x_v[rows, :].astype(f32) + jnp.dot(
                h0_v[rows, :], wd0[...], preferred_element_type=f32)
            return carry

        lax.fori_loop(0, NB, phase_b, 0)
        for c in c_copies:
            c.wait()

        scale = DH ** -0.5

        def attention(i, r0, prev):
            n = 8
            never = i < 0
            q = [q_s[c, pl.ds(r0, n), :] for c in range(NC)]
            if prev is not None:
                q = [jnp.where(never, prev, t) for t in q]
            ls = []
            last = None
            for w in range(W):
                if w and w % (W // qk_st) == 0:
                    q = [jnp.where(never, last, t) for t in q]
                off = HALO + r0 - DIL * w
                p = q[0] * k_s[0, pl.ds(off, n), :]
                for c in range(1, NC):
                    p = p + q[c] * k_s[c, pl.ds(off, n), :]
                last = p
                p = p + pltpu.roll(p, 64, 1)
                p = p + pltpu.roll(p, 32, 1)
                p = p * scale
                if w > 0 and r0 < DIL * w:
                    pos = i * TM + r0 + lax.broadcasted_iota(jnp.int32, (n, 128), 0)
                    p = jnp.where(pos >= DIL * w, p, -1e9)
                ls.append(p)
            m = functools.reduce(jnp.maximum, ls)
            es = [jnp.exp(l - m) for l in ls]
            inv = 1.0 / functools.reduce(jnp.add, es)
            ps = [e * inv for e in es]
            outs = []
            for c in range(NC):
                if c and c % (NC // pv_st) == 0:
                    ps = [jnp.where(never, outs[-1], t) for t in ps]
                o = ps[0] * v_s[c, pl.ds(HALO + r0, n), :]
                for w in range(1, W):
                    o = o + ps[w] * v_s[c, pl.ds(HALO + r0 - DIL * w, n), :]
                outs.append(o)
            return outs

        def main(i, carry):
            rows = blk(i)
            xn = xn_v[rows, :]
            q = jnp.dot(xn, wqkv_p[:, pl.ds(0, D)], preferred_element_type=f32)
            for c in range(NC):
                q_s[c] = q[:, c * 128:(c + 1) * 128]
            k = jnp.dot(xn, wqkv_p[:, pl.ds(D, D)], preferred_element_type=f32)
            for c in range(NC):
                k_s[c, pl.ds(0, HALO), :] = k_s[c, pl.ds(TM, HALO), :]
                k_s[c, pl.ds(HALO, TM), :] = k[:, c * 128:(c + 1) * 128]
            v = jnp.dot(xn, wqkv_p[:, pl.ds(2 * D, D)], preferred_element_type=f32)
            for c in range(NC):
                vc = v[:, c * 128:(c + 1) * 128]
                first = jnp.broadcast_to(vc[0:1, :], (HALO, 128))
                v_s[c, pl.ds(0, HALO), :] = jnp.where(i == 0, first, v_s[c, pl.ds(TM, HALO), :])
                v_s[c, pl.ds(HALO, TM), :] = vc
            prev = None
            for r0 in range(0, TM, 16):
                oa = attention(i, r0, prev)
                ob = attention(i, r0 + 8, oa[-1])
                prev = ob[-1]
                for c in range(NC):
                    o_s[pl.ds(r0, 16), pl.ds(c * 128, 128)] = jnp.concatenate([oa[c], ob[c]], axis=0).astype(bf16)
            for c in range(NCH):
                cols = pl.ds(c * TF, TF)
                g = jnp.dot(xn, wg1[:, cols], preferred_element_type=f32)
                u = jnp.dot(xn, wu1[:, cols], preferred_element_type=f32)
                h_s[:, pl.ds(c * TF, TF)] = (_gelu(g) * u).astype(bf16)
            y = acc_v[rows, :] + jnp.dot(h_s[...], wd1[...], preferred_element_type=f32)
            y = y + jnp.dot(o_s[...], wo_p[...], preferred_element_type=f32)
            out_v[rows, :] = y.astype(bf16)
            o_copy(i).start()
            return carry

        lax.fori_loop(0, NB, main, 0)
        for i in range(NB):
            o_copy(i).wait()

    def f(A_x, A_wqkv, A_wo, B_x, B_w_gate, B_w_up, B_w_down):
        x = A_x.reshape(S, D)
        anyspec = pl.BlockSpec(memory_space=pl.ANY)
        dma = pltpu.SemaphoreType.DMA
        out = pl.pallas_call(
            kern,
            in_specs=[anyspec] * 6,
            out_specs=anyspec,
            out_shape=jax.ShapeDtypeStruct((S, D), bf16),
            scratch_shapes=[
                pltpu.VMEM((S, D), bf16), pltpu.VMEM((S, D), bf16), pltpu.VMEM((S, D), f32),
                pltpu.VMEM((D, 3 * D), bf16), pltpu.VMEM((D, 3 * D), bf16),
                pltpu.VMEM((NC, D, 128), bf16), pltpu.VMEM((H * WST, 128), f32), pltpu.VMEM((D, D), bf16),
                pltpu.VMEM((D, 2 * FA), bf16),
                pltpu.VMEM((D, TF0 - FA), bf16), pltpu.VMEM((D, TF0 - FA), bf16), pltpu.VMEM((TF0, D), bf16),
                pltpu.VMEM((D, FR), bf16), pltpu.VMEM((D, FR), bf16), pltpu.VMEM((FR, D), bf16),
                pltpu.VMEM((S, TF0), bf16),
                pltpu.VMEM((NC, TM, 128), f32), pltpu.VMEM((NC, TM + HALO, 128), f32),
                pltpu.VMEM((NC, TM + HALO, 128), f32),
                pltpu.VMEM((TM, D), bf16), pltpu.VMEM((TM, FR), bf16), pltpu.VMEM((S, D), bf16),
                dma((NB,)), dma((NB,)), dma((NB,)), dma((8,)), dma((NB,)),
            ],
            compiler_params=pltpu.CompilerParams(vmem_limit_bytes=120 * 1024 * 1024, disable_bounds_checks=nobc),
        )(x, A_wqkv, A_wo, B_w_gate, B_w_up, B_w_down)
        return out.reshape(1, S, D)
    return f


@jax.jit
def pallas_parallel_sum__sliding_local_dilated__glu_gated_geglu__prompt_kernel(
    A_x, A_wqkv, A_wo, B_x, B_w_gate, B_w_up, B_w_down):
    return build()(A_x, A_wqkv, A_wo, B_x, B_w_gate, B_w_up, B_w_down)
```

```python
import functools
import numpy as np
import jax
import jax.numpy as jnp
from jax import lax
from jax.experimental import pallas as pl
from jax.experimental.pallas import tpu as pltpu

S, D, F = 2048, 1024, 3584
H, DH, W, DIL = 32, 32, 8, 2
HALO = 16
NC = D // 128
HS, HD = S // 2, D // 2
FC = 512
HC = FC // 2
NCH = F // FC
f32, bf16, u32 = jnp.float32, jnp.bfloat16, jnp.uint32


def _gelu(x):
    c = float(np.sqrt(2.0 / np.pi))
    return x * (0.5 * (1.0 + jnp.tanh(c * (x + 0.044715 * (x * x * x)))))


def _lhs_terms(a11, a12, a21, a22):
    return (a11 + a22, a21 + a22, a11, a22, a11 + a12, a21 - a11, a12 - a22)


def _rhs_terms(b11, b12, b21, b22):
    return (b11 + b22, b11, b12 - b22, b21 - b11, b22, b11 + b12, b21 + b22)


def _product(m):
    m1, m4 = m(0), m(3)
    c11 = m1 + m4
    m2 = m(1)
    c21 = m2 + m4
    c22 = m1 - m2
    m3 = m(2)
    c22 = c22 + m3
    m5 = m(4)
    c12 = m3 + m5
    c11 = c11 - m5
    c11 = c11 + m(6)
    c22 = c22 + m(5)
    return c11, c12, c21, c22


def _ds(start, size, align):
    if isinstance(start, int):
        return pl.ds(start, size)
    return pl.ds(pl.multiple_of(start, align), size)


def build(G=16, M1=128, M2=256, M3=512, M4=256, AG=6, qk_st=8, pv_st=8, scopes=False, nobc=False, PR=16, PG=16, qgate=1, c1=1, q_per=1, slow2=True, gu_per=5, d_per=8, ogate=False, gap=64, late=1, MQ=256, c2=False):
    N1, N2, N3, N4 = HS // M1, HS // M2, HS // M3, HS // M4
    assert N2 == NC // 2
    K1 = HD // N1

    import contextlib
    scope = jax.named_scope if scopes else (lambda n: contextlib.nullcontext())

    def kern(x_hbm, wqkv_hbm, wo_hbm, wg_hbm, wu_hbm, wd_hbm, out_hbm,
             x_v, xa, ha, ha_last, oa, acc, q_s, k_s, v_s,
             bq, bkv, bo, bgu, bd, bd_last, rqkv, ro, ro_f, rg, ru, rd,
             xsem, qsem, gsem, usem, dsem, osem, wosem):

        def x_copy(i):
            rows = _ds(i * 2 * M1, 2 * M1, 2 * M1)
            return pltpu.make_async_copy(x_hbm.at[rows], x_v.at[rows], xsem.at[i])

        def qkv_copy(i):
            rows = _ds(i * K1, K1, K1)
            return pltpu.make_async_copy(wqkv_hbm.at[:, rows, pl.ds(0, D)], rqkv.at[:, rows, pl.ds(0, D)], qsem.at[i])

        kv_copy = pltpu.make_async_copy(wqkv_hbm.at[:, :, pl.ds(D, 2 * D)], rqkv.at[:, :, pl.ds(D, 2 * D)], wosem.at[1])

        def g_copy(c):
            return pltpu.make_async_copy(wg_hbm.at[:, _ds(c * FC, FC, FC)], rg.at[c % 2], gsem.at[c % 2])

        def u_copy(c):
            return pltpu.make_async_copy(wu_hbm.at[:, _ds(c * FC, FC, FC)], ru.at[c % 2], usem.at[c % 2])

        def d_copy(c):
            return pltpu.make_async_copy(wd_hbm.at[_ds(c * FC, FC, FC)], rd.at[c % 2], dsem.at[c % 2])

        wo_copy = pltpu.make_async_copy(wo_hbm, ro, wosem.at[0])

        def out_copy(i):
            rows = _ds(i * 2 * M4, 2 * M4, 2 * M4)
            return pltpu.make_async_copy(x_v.at[rows], out_hbm.at[rows], osem.at[i])

        ha_j = lambda j: ha.at[j] if j < 6 else ha_last
        bd_j = lambda c, j: bd.at[c % 2, j] if j < 6 else bd_last.at[c % 2]

        class Chain:
            def __init__(self, never):
                self.never, self.last = never, None

            def gate(self, t):
                if self.never is None or self.last is None:
                    return t
                last = self.last if self.last.dtype == t.dtype else pltpu.bitcast(self.last, t.dtype)
                if last.shape != t.shape:
                    last = jnp.tile(last, (t.shape[0] // 8, t.shape[1] // 128))
                return jnp.where(self.never, last, t)

            def done(self, t, slow=False):
                if self.never is not None:
                    t = t[:8, :128]
                    self.last = pltpu.roll(t, 1, 1) if slow else t

        def rhs_piece(chain, slow, b11, b12, b21, b22):
            terms = _rhs_terms(chain.gate(b11), b12, b21, chain.gate(b22))
            chain.done(terms[0], slow)
            return [t.astype(bf16) for t in terms]

        def layernorm(i, chain):
            for g in range(M1 // G):
                x = chain.gate(x_v[_ds(i * 2 * M1 + 2 * G * g, 2 * G, G), :].astype(f32))
                mean = jnp.mean(x, axis=-1, keepdims=True)
                xc = x - mean
                var = jnp.mean(xc * xc, axis=-1, keepdims=True)
                xn = xc * lax.rsqrt(var + 1e-5)
                terms = _lhs_terms(xn[:G, :HD], xn[:G, HD:], xn[G:, :HD], xn[G:, HD:])
                for j, t in enumerate(terms):
                    xa[j, _ds(i * M1 + G * g, G, G), :] = t.astype(bf16)
                chain.done(terms[0])
                yield

        def prep_qkv(i, n, parts, chain):
            lane = lax.broadcasted_iota(jnp.int32, (PR // 2, 128), 1)
            grp = (lane >> 2) & 7
            for r in range(0, HD // n, PR):
                rows = _ds(i * (HD // n) + r, PR, PR)
                for part in parts:
                    halves = []
                    for half in range(2):
                        a = []
                        for cs in range(NC):
                            cd = (grp - cs) & 7
                            dl = ((lane >> 5) - (grp < cd).astype(jnp.int32)) & 3
                            idx = (lane & 3) * 32 + cd * 4 + dl
                            w = pltpu.bitcast(rqkv[half, rows, pl.ds(part * D + cs * 128, 128)], u32)
                            a.append(jnp.take_along_axis(chain.gate(w), idx, axis=1))
                        a = [a[(-j) % 8] for j in range(8)]
                        for b in (1, 2, 4):
                            sel = (grp & b) != 0
                            a = [jnp.where(sel, a[(j - b) % 8], a[j]) for j in range(8)]
                        a = [a[cd] if cd == 0 else pltpu.roll(a[cd], 128 - 4 * cd, 1) for cd in range(NC)]
                        halves.append(a)
                    if qgate == 0:
                        chain.done(halves[1][-1])
                    for c in range(0, NC // 2, 2):
                        ld = lambda half, cc: pltpu.bitcast(
                            jnp.concatenate(halves[half][cc:cc + 2], axis=1), bf16).astype(f32)
                        terms = _rhs_terms(ld(0, c), ld(0, c + 4), ld(1, c), ld(1, c + 4))
                        for j, t in enumerate(terms):
                            (bq if part == 0 else bkv.at[part - 1])[j, rows, pl.ds(c * 128, 256)] = t.astype(bf16)
                    if qgate == 1:
                        chain.done(terms[0])
                    yield

        def prep_wo(i, chain, slow):
            for half in range(2):
                cols = _ds((i + 4 * half) * 128, 128, 128)
                for h in range(H):
                    t = chain.gate(ro[pl.ds(h * DH, DH), cols].astype(f32))
                    ro_f[half, pl.ds(h * (DH + 1), DH), :] = t
                    chain.done(t, slow and h % 4 == 3)
                    yield
            for d in range(DH // 2):
                ld = lambda half, dd: ro_f[half, pl.ds(dd, H, stride=DH + 1), :]
                terms = rhs_piece(chain, slow, ld(0, d), ld(1, d), ld(0, d + DH // 2), ld(1, d + DH // 2))
                for j, t in enumerate(terms):
                    bo[j, pl.ds(d * H, H), _ds(i * 128, 128, 128)] = t
                yield

        def prep_gu(c, i, n, chain, slow):
            kp = HD // n
            for r in range(0, kp, PG):
                lo, hi = _ds(i * kp + r, PG, PG), _ds(HD + i * kp + r, PG, PG)
                for off, raw in ((0, rg), (HC, ru)):
                    ld = lambda rr, o: raw[c % 2, rr, pl.ds(o, HC)].astype(f32)
                    terms = rhs_piece(chain, slow, ld(lo, 0), ld(lo, HC), ld(hi, 0), ld(hi, HC))
                    for j, t in enumerate(terms):
                        bgu[c % 2, j, lo, pl.ds(off, HC)] = t
                    yield

        def prep_d(c, i, n, chain, slow):
            kp = HC // n
            for r in range(0, kp, PG):
                lo, hi = _ds(i * kp + r, PG, PG), _ds(HC + i * kp + r, PG, PG)
                for o in range(0, HD, 256):
                    ld = lambda rr, oo: rd[c % 2, rr, pl.ds(oo + o, 256)].astype(f32)
                    terms = rhs_piece(chain, slow, ld(lo, 0), ld(lo, HD), ld(hi, 0), ld(hi, HD))
                    for j, t in enumerate(terms):
                        bd_j(c, j)[lo, pl.ds(o, 256)] = t
                    yield

        def run(*jobs):
            jobs = list(jobs)
            while jobs:
                for job in list(jobs):
                    gen, n = job
                    for _ in range(n):
                        if next(gen, "end") == "end":
                            jobs.remove(job)
                            break

        def gate_up(c, rows, before_store=None):
            quads = _product(lambda j: jnp.dot(xa[j, rows, :], bgu[c % 2, j], preferred_element_type=f32))
            hs = [_gelu(t[:, :HC]) * t[:, HC:] for t in quads]
            if before_store is not None:
                before_store()
            for j, t in enumerate(_lhs_terms(*hs)):
                ha_j(j)[rows, :] = t.astype(bf16)

        log2e = float(np.log2(np.e))
        scale = DH ** -0.5

        def attention8(base, r, chain, outs):
            q = [q_s[c, _ds(base + r, 8, 8), :] for c in range(NC)]
            ls = []
            for w in range(W):
                if w % (W // qk_st) == 0:
                    q = [chain.gate(t) for t in q]
                at = pl.ds(base + (HALO + r - DIL * w), 8)
                p = q[0] * k_s[0, at, :]
                for c in range(1, NC):
                    p = p + q[c] * k_s[c, at, :]
                chain.done(p)
                p = p + pltpu.roll(p, 64, 1)
                p = p + pltpu.roll(p, 32, 1)
                if r < DIL * w:
                    pos = base + r + lax.broadcasted_iota(jnp.int32, (8, 128), 0)
                    p = jnp.where(pos >= DIL * w, p, -1e9 * log2e)
                ls.append(p)
                yield
            m = functools.reduce(jnp.maximum, ls)
            ps = [jnp.exp2(l - m) for l in ls]
            inv = 1.0 / functools.reduce(jnp.add, ps)
            for n, c in enumerate((0, 1, 4, 5, 2, 3, 6, 7)):
                if n and n % (NC // pv_st) == 0:
                    ps = [chain.gate(t) for t in ps]
                o = ps[0] * v_s[c, pl.ds(base + (HALO + r), 8), :]
                for w in range(1, W):
                    o = o + ps[w] * v_s[c, pl.ds(base + (HALO + r - DIL * w), 8), :]
                chain.done(o)
                outs[c] = o * inv
                yield

        def attention(g0, chain):
            base = g0 * (2 * G)
            for g in range(AG):
                parts = []
                for r in range(2 * G * g, 2 * G * (g + 1), 8):
                    parts.append({})
                    yield from attention8(base, r, chain, parts[-1])
                n = G // 8
                quad = lambda p, c: jnp.concatenate(
                    [jnp.concatenate([parts[p * n + t][c], parts[p * n + t][c + 1]], axis=1) for t in range(n)], axis=0)
                for c in range(0, NC // 2, 2):
                    terms = _lhs_terms(quad(0, c), quad(0, c + 4), quad(1, c), quad(1, c + 4))
                    for j, t in enumerate(terms):
                        oa[j, _ds((g0 + g) * G, G, G), pl.ds(c * 128, 256)] = t.astype(bf16)
                    if ogate:
                        chain.done(terms[0])

        x_copy(0).start()
        g_copy(0).start()
        u_copy(0).start()
        x_copy(1).start()
        qkv_copy(0).start()
        with scope("s0_x0"):
            x_copy(0).wait()
        with scope("s1_ln0"):
            run((layernorm(0, Chain(None)), 1))
        with scope("s2_gu0"):
            g_copy(0).wait()
            u_copy(0).wait()
        with scope("s3_prep0"):
            run((prep_gu(0, 0, 1, Chain(None), False), 1))

        def stage1(i, carry):
            pl.when(i + 2 < N1)(x_copy(jnp.minimum(i + 2, N1 - 1)).start)
            pl.when(i + 1 < N1)(qkv_copy(jnp.minimum(i + 1, N1 - 1)).start)
            pl.when(i == 1)(kv_copy.start)
            nxt = jnp.minimum(i + 1, N1 - 1)
            pl.when(i + 1 < N1)(x_copy(nxt).wait)
            qkv_copy(i).wait()
            gate_up(0, _ds(i * M1, M1, M1))
            ca = Chain(i < 0 if c1 in (1, 3) else None)
            cb = ca if c1 == 3 else Chain(i < 0 if c1 in (1, 2) else None)
            run((layernorm(nxt, ca), 1), (prep_qkv(i, N1, (0,), cb), q_per))
            return carry

        with scope("s4_stage1"):
            lax.fori_loop(0, N1, stage1, 0)

        def project(i, m, terms, dst, off, mult=None):
            rows = _ds(i * m, m, m)
            quads = _product(lambda j: jnp.dot(xa[j, rows, :], terms[j], preferred_element_type=f32))
            for k, t in enumerate(quads):
                if mult is not None:
                    t = t * mult
                for g in range(m // G):
                    at = _ds(i * 2 * m + (off + 2 * G * g + G * (k // 2)), G, G)
                    for c in range(NC // 2):
                        dst[c + 4 * (k % 2), at, :] = t[G * g:G * (g + 1), c * 128:(c + 1) * 128]

        for cp in (wo_copy, d_copy(0), g_copy(1), u_copy(1)):
            cp.start()
        with scope("s5_wait"):
            kv_copy.wait()

        def stage2q(i, carry):
            project(i, MQ, bq, q_s, 0, scale * log2e)
            run((prep_qkv(i, HS // MQ, (1, 2), Chain(i < 0 if c2 else None)), 1))
            return carry

        with scope("s6_stage2q"):
            lax.fori_loop(0, HS // MQ, stage2q, 0)
        for cp in (d_copy(1), g_copy(2), u_copy(2)):
            cp.start()
        for cp in (wo_copy, d_copy(0), g_copy(1), u_copy(1)):
            cp.wait()

        def stage2kv(i, carry):
            project(i, M2, bkv.at[0], k_s, HALO)
            project(i, M2, bkv.at[1], v_s, HALO)
            chain = Chain(i < 0)
            run((prep_wo(i, chain, slow2), 1000), (prep_d(0, i, N2, chain, slow2), 1000), (prep_gu(1, i, N2, chain, slow2), 1000))
            return carry

        with scope("s6_stage2kv"):
            lax.fori_loop(0, N2, stage2kv, 0)
        for c in range(NC):
            k_s[c, pl.ds(0, HALO), :] = jnp.zeros((HALO, 128), f32)
            v_s[c, pl.ds(0, HALO), :] = jnp.broadcast_to(v_s[c, pl.ds(HALO, 1), :], (HALO, 128))

        def stage3(t, carry):
            c, i = t // N3, t % N3

            @pl.when(i == 0)
            def _():
                pl.when(c + 2 < NCH)(d_copy(jnp.minimum(c + 2, NCH - 1)).start)
                pl.when(c + 3 < NCH)(g_copy(jnp.minimum(c + 3, NCH - 1)).start)
                pl.when(c + 3 < NCH)(u_copy(jnp.minimum(c + 3, NCH - 1)).start)
                d_copy(c + 1).wait()
                pl.when(c + 2 < NCH)(g_copy(jnp.minimum(c + 2, NCH - 1)).wait)
                pl.when(c + 2 < NCH)(u_copy(jnp.minimum(c + 2, NCH - 1)).wait)

            rows = _ds(i * M3, M3, M3)
            def down(j):
                acc[j, rows, :] = jnp.where(c > 0, acc[j, rows, :], 0.0) + jnp.dot(
                    ha_j(j)[rows, :], bd_j(c, j)[...], preferred_element_type=f32)

            for j in range(7 - late):
                down(j)
            chain = Chain(t < 0)
            att = attention(jnp.minimum(t * AG, HS // G - AG), chain)
            for _ in prep_gu(c + 2, i, N3, chain, False):
                for _ in range(gu_per):
                    next(att)
            gate_up(c + 1, rows, (lambda: down(6)) if late else None)
            for _ in range(gap):
                next(att)
            run((prep_d(c + 1, i, N3, chain, False), 1), (att, d_per))
            return carry

        with scope("s7_stage3"):
            lax.fori_loop(0, (NCH - 1) * N3, stage3, 0)

        def stage4(i, carry):
            rows = _ds(i * M4, M4, M4)
            quads = _product(
                lambda j: acc[j, rows, :]
                + jnp.dot(ha_j(j)[rows, :], bd_j(NCH - 1, j)[...], preferred_element_type=f32)
                + jnp.dot(oa[j, rows, :], bo[j], preferred_element_type=f32))
            for k, t in enumerate(quads):
                for g in range(M4 // G):
                    at = _ds(i * 2 * M4 + (2 * G * g + G * (k // 2)), G, G)
                    cols = pl.ds((k % 2) * HD, HD)
                    x_v[at, cols] = (x_v[at, cols].astype(f32) + t[G * g:G * (g + 1)]).astype(bf16)
            out_copy(i).start()
            return carry

        with scope("s8_stage4"):
            lax.fori_loop(0, N4, stage4, 0)
        with scope("s9_tail"):
            for i in range(N4):
                out_copy(i).wait()

    def f(A_x, A_wqkv, A_wo, B_x, B_w_gate, B_w_up, B_w_down):
        anyspec = pl.BlockSpec(memory_space=pl.ANY)
        dma = pltpu.SemaphoreType.DMA
        vmem = pltpu.VMEM
        out = pl.pallas_call(
            kern,
            in_specs=[anyspec] * 6,
            out_specs=anyspec,
            out_shape=jax.ShapeDtypeStruct((S, D), bf16),
            scratch_shapes=[
                vmem((S, D), bf16), vmem((7, HS, HD), bf16), vmem((6, HS, HC), bf16), vmem((HS, HC), bf16), vmem((7, HS, HD), bf16),
                vmem((7, HS, HD), f32),
                vmem((NC, S, 128), f32), vmem((NC, S + HALO, 128), f32), vmem((NC, S + HALO, 128), f32),
                vmem((7, HD, HD), bf16), vmem((2, 7, HD, HD), bf16), vmem((7, HD, HD), bf16),
                vmem((2, 7, HD, FC), bf16), vmem((2, 6, HC, HD), bf16), vmem((2, HC, HD), bf16),
                vmem((2, HD, 3 * D), bf16), vmem((D, D), bf16), vmem((2, H * (DH + 1), 128), f32),
                vmem((2, D, FC), bf16), vmem((2, D, FC), bf16), vmem((2, FC, D), bf16),
                dma((N1,)), dma((N1,)), dma((2,)), dma((2,)), dma((2,)), dma((N4,)), dma((2,)),
            ],
            compiler_params=pltpu.CompilerParams(vmem_limit_bytes=124 * 1024 * 1024, disable_bounds_checks=nobc),
        )(A_x.reshape(S, D), A_wqkv.reshape(2, HD, 3 * D), A_wo, B_w_gate, B_w_up, B_w_down)
        return out.reshape(1, S, D)
    return f


@jax.jit
def pallas_parallel_sum__sliding_local_dilated__glu_gated_geglu__prompt_kernel(
    A_x, A_wqkv, A_wo, B_x, B_w_gate, B_w_up, B_w_down):
    return build()(A_x, A_wqkv, A_wo, B_x, B_w_gate, B_w_up, B_w_down)
```

```python
import functools
import numpy as np
import jax
import jax.numpy as jnp
from jax import lax
from jax.experimental import pallas as pl
from jax.experimental.pallas import tpu as pltpu

S, D, F = 2048, 1024, 3584
H, DH, W, DIL = 32, 32, 8, 2
HALO = 16
NC = D // 128
HS, HD = S // 2, D // 2
FC = 512
HC = FC // 2
NCH = F // FC
f32, bf16, u32 = jnp.float32, jnp.bfloat16, jnp.uint32


def _gelu(x):
    c = float(np.sqrt(2.0 / np.pi))
    return x * (0.5 * (1.0 + jnp.tanh(c * (x + 0.044715 * (x * x * x)))))


def _lhs_terms(a11, a12, a21, a22):
    return (a11 + a22, a21 + a22, a11, a22, a11 + a12, a21 - a11, a12 - a22)


def _rhs_terms(b11, b12, b21, b22):
    return (b11 + b22, b11, b12 - b22, b21 - b11, b22, b11 + b12, b21 + b22)


def _product(m):
    m1, m4 = m(0), m(3)
    c11 = m1 + m4
    m2 = m(1)
    c21 = m2 + m4
    c22 = m1 - m2
    m3 = m(2)
    c22 = c22 + m3
    m5 = m(4)
    c12 = m3 + m5
    c11 = c11 - m5
    c11 = c11 + m(6)
    c22 = c22 + m(5)
    return c11, c12, c21, c22


def _ds(start, size, align):
    if isinstance(start, int):
        return pl.ds(start, size)
    return pl.ds(pl.multiple_of(start, align), size)


def build(G=16, M1=128, M2=256, M3=512, M4=256, AG=6, qk_st=8, pv_st=8, scopes=False, nobc=False, PR=16, PG=16, qgate=1, c1=1, q_per=1, slow2=True, gu_per=5, d_per=8, ogate=False, gap=64, late=1, MQ=256, c2=False,
          gmode='half', qk_done=0, sm_st=2, sm_done=0, pv_done=0, pv_slow=0, only=None):
    N1, N2, N3, N4 = HS // M1, HS // M2, HS // M3, HS // M4
    assert N2 == NC // 2
    K1 = HD // N1

    import contextlib
    scope = jax.named_scope if scopes else (lambda n: contextlib.nullcontext())

    def kern(x_hbm, wqkv_hbm, wo_hbm, wg_hbm, wu_hbm, wd_hbm, out_hbm,
             x_v, xa, ha, ha_last, oa, acc, q_s, k_s, v_s,
             bq, bkv, bo, bgu, bd, bd_last, rqkv, ro, ro_f, rg, ru, rd,
             xsem, qsem, kvsem, gsem, usem, dsem, osem, wosem):

        def x_copy(i):
            rows = _ds(i * 2 * M1, 2 * M1, 2 * M1)
            return pltpu.make_async_copy(x_hbm.at[rows], x_v.at[rows], xsem.at[i])

        def qkv_copy(i):
            rows = _ds(i * K1, K1, K1)
            return pltpu.make_async_copy(wqkv_hbm.at[:, rows, pl.ds(0, D)], rqkv.at[:, rows, pl.ds(0, D)], qsem.at[i])

        def kv_copy(i):
            rows = _ds(i * K1, K1, K1)
            return pltpu.make_async_copy(
                wqkv_hbm.at[:, rows, pl.ds(D, 2 * D)], rqkv.at[:, rows, pl.ds(D, 2 * D)], kvsem.at[i])

        def g_copy(c):
            return pltpu.make_async_copy(wg_hbm.at[:, _ds(c * FC, FC, FC)], rg.at[c % 2], gsem.at[c % 2])

        def u_copy(c):
            return pltpu.make_async_copy(wu_hbm.at[:, _ds(c * FC, FC, FC)], ru.at[c % 2], usem.at[c % 2])

        def d_copy(c):
            return pltpu.make_async_copy(wd_hbm.at[_ds(c * FC, FC, FC)], rd.at[c % 2], dsem.at[c % 2])

        wo_copy = pltpu.make_async_copy(wo_hbm, ro, wosem.at[0])

        def out_copy(i):
            rows = _ds(i * 2 * M4, 2 * M4, 2 * M4)
            return pltpu.make_async_copy(x_v.at[rows], out_hbm.at[rows], osem.at[i])

        def get(ref, rows=None):
            at = slice(None) if rows is None else _ds(rows[0] // 2, rows[1] // 2, rows[1] // 2)
            return pltpu.bitcast(ref[at, :], bf16)

        def put(ref, rows, c0, t):
            at = _ds(rows[0] // 2, rows[1] // 2, rows[1] // 2)
            ref[at, _ds(c0 * 128, t.shape[1], 128)] = pltpu.bitcast(t.astype(bf16), u32)

        ha_j = lambda j: ha.at[j] if j < 6 else ha_last
        bd_j = lambda c, j: bd.at[c % 2, j] if j < 6 else bd_last.at[c % 2]

        class Chain:
            def __init__(self, never):
                self.never, self.last = never, None

            def gate(self, t):
                if self.never is None or self.last is None:
                    return t
                last = self.last if self.last.dtype == t.dtype else pltpu.bitcast(self.last, t.dtype)
                if last.shape != t.shape:
                    last = jnp.tile(last, (t.shape[0] // 8, t.shape[1] // 128))
                return jnp.where(self.never, last, t)

            def done(self, t, slow=False):
                if self.never is not None:
                    t = t[:8, :128]
                    self.last = pltpu.roll(t, 1, 1) if slow else t

        def rhs_piece(chain, slow, b11, b12, b21, b22):
            terms = _rhs_terms(chain.gate(b11), b12, b21, chain.gate(b22))
            chain.done(terms[0], slow)
            return terms

        def layernorm(i, chain):
            for g in range(M1 // G):
                x = chain.gate(x_v[_ds(i * 2 * M1 + 2 * G * g, 2 * G, G), :].astype(f32))
                mean = jnp.mean(x, axis=-1, keepdims=True)
                xc = x - mean
                var = jnp.mean(xc * xc, axis=-1, keepdims=True)
                xn = xc * lax.rsqrt(var + 1e-5)
                terms = _lhs_terms(xn[:G, :HD], xn[:G, HD:], xn[G:, :HD], xn[G:, HD:])
                for j, t in enumerate(terms):
                    put(xa.at[j], (i * M1 + G * g, G), 0, t)
                chain.done(terms[0])
                yield

        def prep_qkv(i, n, parts, chain):
            lane = lax.broadcasted_iota(jnp.int32, (PR // 2, 128), 1)
            grp = (lane >> 2) & 7
            for r in range(0, HD // n, PR):
                rows = _ds(i * (HD // n) + r, PR, PR)
                for part in parts:
                    halves = []
                    for half in range(2):
                        a = []
                        for cs in range(NC):
                            cd = (grp - cs) & 7
                            dl = ((lane >> 5) - (grp < cd).astype(jnp.int32)) & 3
                            idx = (lane & 3) * 32 + cd * 4 + dl
                            w = pltpu.bitcast(rqkv[half, rows, pl.ds(part * D + cs * 128, 128)], u32)
                            a.append(jnp.take_along_axis(chain.gate(w), idx, axis=1))
                        a = [a[(-j) % 8] for j in range(8)]
                        for b in (1, 2, 4):
                            sel = (grp & b) != 0
                            a = [jnp.where(sel, a[(j - b) % 8], a[j]) for j in range(8)]
                        a = [a[cd] if cd == 0 else pltpu.roll(a[cd], 128 - 4 * cd, 1) for cd in range(NC)]
                        halves.append(a)
                    if qgate == 0:
                        chain.done(halves[1][-1])
                    for c in range(0, NC // 2, 2):
                        ld = lambda half, cc: pltpu.bitcast(
                            jnp.concatenate(halves[half][cc:cc + 2], axis=1), bf16).astype(f32)
                        terms = _rhs_terms(ld(0, c), ld(0, c + 4), ld(1, c), ld(1, c + 4))
                        for j, t in enumerate(terms):
                            put(bq.at[j] if part == 0 else bkv.at[part - 1, j], (i * (HD // n) + r, PR), c, t)
                    if qgate == 1:
                        chain.done(terms[0])
                    yield

        def prep_wo(i, chain, slow):
            for half in range(2):
                cols = _ds((i + 4 * half) * 128, 128, 128)
                for h in range(H):
                    t = chain.gate(ro[pl.ds(h * DH, DH), cols].astype(f32))
                    ro_f[half, pl.ds(h * (DH + 1), DH), :] = t
                    chain.done(t, slow and h % 4 == 3)
                    yield
            for d in range(DH // 2):
                ld = lambda half, dd: ro_f[half, pl.ds(dd, H, stride=DH + 1), :]
                terms = rhs_piece(chain, slow, ld(0, d), ld(1, d), ld(0, d + DH // 2), ld(1, d + DH // 2))
                for j, t in enumerate(terms):
                    put(bo.at[j], (d * H, H), i, t)
                yield

        def prep_gu(c, i, n, chain, slow):
            kp = HD // n
            for r in range(0, kp, PG):
                lo, hi = _ds(i * kp + r, PG, PG), _ds(HD + i * kp + r, PG, PG)
                for off, raw in ((0, rg), (HC, ru)):
                    ld = lambda rr, o: raw[c % 2, rr, pl.ds(o, HC)].astype(f32)
                    terms = rhs_piece(chain, slow, ld(lo, 0), ld(lo, HC), ld(hi, 0), ld(hi, HC))
                    for j, t in enumerate(terms):
                        put(bgu.at[c % 2, j], (i * kp + r, PG), off // 128, t)
                    yield

        def prep_d(c, i, n, chain, slow):
            kp = HC // n
            for r in range(0, kp, PG):
                lo, hi = _ds(i * kp + r, PG, PG), _ds(HC + i * kp + r, PG, PG)
                for o in range(0, HD, 256):
                    ld = lambda rr, oo: rd[c % 2, rr, pl.ds(oo + o, 256)].astype(f32)
                    terms = rhs_piece(chain, slow, ld(lo, 0), ld(lo, HD), ld(hi, 0), ld(hi, HD))
                    for j, t in enumerate(terms):
                        put(bd_j(c, j), (i * kp + r, PG), o // 128, t)
                    yield

        def run(*jobs):
            jobs = list(jobs)
            while jobs:
                for job in list(jobs):
                    gen, n = job
                    for _ in range(n):
                        if next(gen, "end") == "end":
                            jobs.remove(job)
                            break

        def gate_up(c, rows, before_store=None):
            quads = _product(lambda j: jnp.dot(get(xa.at[j], rows), get(bgu.at[c % 2, j]), preferred_element_type=f32))
            hs = [_gelu(t[:, :HC]) * t[:, HC:] for t in quads]
            if before_store is not None:
                before_store()
            for j, t in enumerate(_lhs_terms(*hs)):
                put(ha_j(j), rows, 0, t)

        log2e = float(np.log2(np.e))
        scale = DH ** -0.5

        def attention8(base, r, chain, outs):
            q = [q_s[c, _ds(base + r, 8, 8), :] for c in range(NC)]
            ls = []
            for w in range(W):
                if gmode == "q" and w % (W // qk_st) == 0:
                    q = [chain.gate(t) for t in q]
                if gmode == "half":
                    q = [chain.gate(t) if c % 2 == w % 2 else t for c, t in enumerate(q)]
                at = pl.ds(base + (HALO + r - DIL * w), 8)
                p = q[0] * k_s[0, at, :]
                if gmode == "acc":
                    p = chain.gate(p)
                for c in range(1, NC):
                    p = p + q[c] * k_s[c, at, :]
                if qk_done == 0:
                    chain.done(p)
                p = p + pltpu.roll(p, 64, 1)
                if qk_done == 1:
                    chain.done(p)
                p = p + pltpu.roll(p, 32, 1)
                if qk_done == 2:
                    chain.done(p)
                if r < DIL * w:
                    pos = base + r + lax.broadcasted_iota(jnp.int32, (8, 128), 0)
                    p = jnp.where(pos >= DIL * w, p, -1e9 * log2e)
                ls.append(p)
                yield
            m = functools.reduce(jnp.maximum, ls)
            ps = []
            for w, l in enumerate(ls):
                if sm_st and w and w % sm_st == 0:
                    m = jnp.where(chain.never, ps[-1], m)
                ps.append(jnp.exp2(l - m))
            inv = 1.0 / functools.reduce(jnp.add, ps)
            if sm_done:
                chain.done(inv if sm_done == 1 else ps[-1])
                ps = [chain.gate(t) for t in ps]
            for n, c in enumerate((0, 1, 4, 5, 2, 3, 6, 7)):
                if gmode == "q" and n and n % (NC // pv_st) == 0:
                    ps = [chain.gate(t) for t in ps]
                if gmode == "half" and n:
                    ps = [chain.gate(t) if w % 2 == n % 2 else t for w, t in enumerate(ps)]
                o = ps[0] * v_s[c, pl.ds(base + (HALO + r), 8), :]
                if gmode == "acc" and n:
                    o = chain.gate(o)
                for w in range(1, W):
                    o = o + ps[w] * v_s[c, pl.ds(base + (HALO + r - DIL * w), 8), :]
                outs[c] = o * inv
                chain.done(outs[c] if pv_done else o, pv_slow and n % pv_slow == pv_slow - 1)
                yield

        def attention(g0, chain):
            base = g0 * (2 * G)
            for g in range(AG):
                parts = []
                for r in range(2 * G * g, 2 * G * (g + 1), 8):
                    parts.append({})
                    yield from attention8(base, r, chain, parts[-1])
                n = G // 8
                quad = lambda p, c: jnp.concatenate(
                    [jnp.concatenate([parts[p * n + t][c], parts[p * n + t][c + 1]], axis=1) for t in range(n)], axis=0)
                for c in range(0, NC // 2, 2):
                    terms = _lhs_terms(quad(0, c), quad(0, c + 4), quad(1, c), quad(1, c + 4))
                    for j, t in enumerate(terms):
                        put(oa.at[j], ((g0 + g) * G, G), c, t)
                    if ogate:
                        chain.done(terms[0])

        x_copy(0).start()
        g_copy(0).start()
        u_copy(0).start()
        x_copy(1).start()
        qkv_copy(0).start()
        with scope("s0_x0"):
            x_copy(0).wait()
        with scope("s1_ln0"):
            run((layernorm(0, Chain(None)), 1))
        with scope("s2_gu0"):
            g_copy(0).wait()
            u_copy(0).wait()
        with scope("s3_prep0"):
            run((prep_gu(0, 0, 1, Chain(None), False), 1))

        def stage1(i, carry):
            pl.when(i + 2 < N1)(x_copy(jnp.minimum(i + 2, N1 - 1)).start)
            pl.when(i + 1 < N1)(qkv_copy(jnp.minimum(i + 1, N1 - 1)).start)
            kv_copy(i).start()
            nxt = jnp.minimum(i + 1, N1 - 1)
            pl.when(i + 1 < N1)(x_copy(nxt).wait)
            qkv_copy(i).wait()
            gate_up(0, (i * M1, M1))
            ca = Chain(i < 0 if c1 in (1, 3) else None)
            cb = ca if c1 == 3 else Chain(i < 0 if c1 in (1, 2) else None)
            run((layernorm(nxt, ca), 1), (prep_qkv(i, N1, (0,), cb), q_per))
            return carry

        with scope("s4_stage1"):
            if only in (None, 1): lax.fori_loop(0, N1, stage1, 0)

        def project(i, m, terms, dst, off, mult=None):
            rows = (i * m, m)
            quads = _product(lambda j: jnp.dot(get(xa.at[j], rows), get(terms.at[j]), preferred_element_type=f32))
            for k, t in enumerate(quads):
                if mult is not None:
                    t = t * mult
                for g in range(m // G):
                    at = _ds(i * 2 * m + (off + 2 * G * g + G * (k // 2)), G, G)
                    for c in range(NC // 2):
                        dst[c + 4 * (k % 2), at, :] = t[G * g:G * (g + 1), c * 128:(c + 1) * 128]

        for cp in (wo_copy, d_copy(0), g_copy(1), u_copy(1)):
            cp.start()
        with scope("s5_wait"):
            for i in range(N1):
                kv_copy(i).wait()

        def stage2q(i, carry):
            project(i, MQ, bq, q_s, 0, scale * log2e)
            run((prep_qkv(i, HS // MQ, (1, 2), Chain(i < 0 if c2 else None)), 1))
            return carry

        with scope("s6_stage2q"):
            if only in (None, 2): lax.fori_loop(0, HS // MQ, stage2q, 0)
        for cp in (d_copy(1), g_copy(2), u_copy(2)):
            cp.start()
        for cp in (wo_copy, d_copy(0), g_copy(1), u_copy(1)):
            cp.wait()

        def stage2kv(i, carry):
            project(i, M2, bkv.at[0], k_s, HALO)
            project(i, M2, bkv.at[1], v_s, HALO)
            chain = Chain(i < 0)
            run((prep_wo(i, chain, slow2), 1000), (prep_d(0, i, N2, chain, slow2), 1000), (prep_gu(1, i, N2, chain, slow2), 1000))
            return carry

        with scope("s6_stage2kv"):
            if only in (None, 2): lax.fori_loop(0, N2, stage2kv, 0)
        for c in range(NC):
            k_s[c, pl.ds(0, HALO), :] = jnp.zeros((HALO, 128), f32)
            v_s[c, pl.ds(0, HALO), :] = jnp.broadcast_to(v_s[c, pl.ds(HALO, 1), :], (HALO, 128))

        def stage3(t, carry):
            c, i = t // N3, t % N3

            @pl.when(i == 0)
            def _():
                pl.when(c + 2 < NCH)(d_copy(jnp.minimum(c + 2, NCH - 1)).start)
                pl.when(c + 3 < NCH)(g_copy(jnp.minimum(c + 3, NCH - 1)).start)
                pl.when(c + 3 < NCH)(u_copy(jnp.minimum(c + 3, NCH - 1)).start)
                d_copy(c + 1).wait()
                pl.when(c + 2 < NCH)(g_copy(jnp.minimum(c + 2, NCH - 1)).wait)
                pl.when(c + 2 < NCH)(u_copy(jnp.minimum(c + 2, NCH - 1)).wait)

            rows = _ds(i * M3, M3, M3)
            def down(j):
                acc[j, rows, :] = jnp.where(c > 0, acc[j, rows, :], 0.0) + jnp.dot(
                    get(ha_j(j), (i * M3, M3)), get(bd_j(c, j)), preferred_element_type=f32)

            for j in range(7 - late):
                down(j)
            chain = Chain(t < 0)
            att = attention(jnp.minimum(t * AG, HS // G - AG), chain)
            for _ in prep_gu(c + 2, i, N3, chain, False):
                for _ in range(gu_per):
                    next(att)
            gate_up(c + 1, (i * M3, M3), (lambda: down(6)) if late else None)
            for _ in range(gap):
                next(att)
            run((prep_d(c + 1, i, N3, chain, False), 1), (att, d_per))
            return carry

        with scope("s7_stage3"):
            if only in (None, 3): lax.fori_loop(0, (NCH - 1) * N3, stage3, 0)

        def stage4(i, carry):
            rows = _ds(i * M4, M4, M4)
            quads = _product(
                lambda j: acc[j, rows, :]
                + jnp.dot(get(ha_j(j), (i * M4, M4)), get(bd_j(NCH - 1, j)), preferred_element_type=f32)
                + jnp.dot(get(oa.at[j], (i * M4, M4)), get(bo.at[j]), preferred_element_type=f32))
            for k, t in enumerate(quads):
                for g in range(M4 // G):
                    at = _ds(i * 2 * M4 + (2 * G * g + G * (k // 2)), G, G)
                    cols = pl.ds((k % 2) * HD, HD)
                    x_v[at, cols] = (x_v[at, cols].astype(f32) + t[G * g:G * (g + 1)]).astype(bf16)
            out_copy(i).start()
            return carry

        with scope("s8_stage4"):
            if only in (None, 4): lax.fori_loop(0, N4, stage4, 0)
        with scope("s9_tail"):
            for i in range(N4):
                out_copy(i).wait()

    def f(A_x, A_wqkv, A_wo, B_x, B_w_gate, B_w_up, B_w_down):
        anyspec = pl.BlockSpec(memory_space=pl.ANY)
        dma = pltpu.SemaphoreType.DMA
        vmem = pltpu.VMEM
        out = pl.pallas_call(
            kern,
            in_specs=[anyspec] * 6,
            out_specs=anyspec,
            out_shape=jax.ShapeDtypeStruct((S, D), bf16),
            scratch_shapes=[
                vmem((S, D), bf16),
                vmem((7, HS // 2, HD), u32), vmem((6, HS // 2, HC), u32), vmem((HS // 2, HC), u32),
                vmem((7, HS // 2, HD), u32), vmem((7, HS, HD), f32),
                vmem((NC, S, 128), f32), vmem((NC, S + HALO, 128), f32), vmem((NC, S + HALO, 128), f32),
                vmem((7, HD // 2, HD), u32), vmem((2, 7, HD // 2, HD), u32), vmem((7, HD // 2, HD), u32),
                vmem((2, 7, HD // 2, FC), u32), vmem((2, 6, HC // 2, HD), u32), vmem((2, HC // 2, HD), u32),
                vmem((2, HD, 3 * D), bf16), vmem((D, D), bf16), vmem((2, H * (DH + 1), 128), f32),
                vmem((2, D, FC), bf16), vmem((2, D, FC), bf16), vmem((2, FC, D), bf16),
                dma((N1,)), dma((N1,)), dma((N1,)), dma((2,)), dma((2,)), dma((2,)), dma((N4,)), dma((1,)),
            ],
            compiler_params=pltpu.CompilerParams(vmem_limit_bytes=124 * 1024 * 1024, disable_bounds_checks=nobc),
        )(A_x.reshape(S, D), A_wqkv.reshape(2, HD, 3 * D), A_wo, B_w_gate, B_w_up, B_w_down)
        return out.reshape(1, S, D)
    return f


@jax.jit
def pallas_parallel_sum__sliding_local_dilated__glu_gated_geglu__prompt_kernel(
    A_x, A_wqkv, A_wo, B_x, B_w_gate, B_w_up, B_w_down):
    return build()(A_x, A_wqkv, A_wo, B_x, B_w_gate, B_w_up, B_w_down)
```

```python
import functools
import numpy as np
import jax
import jax.numpy as jnp
from jax import lax
from jax.experimental import pallas as pl
from jax.experimental.pallas import tpu as pltpu

S, D, F = 2048, 1024, 3584
H, DH, W, DIL = 32, 32, 8, 2
HALO = 16
NC = D // 128
HS, HD = S // 2, D // 2
FC = 512
HC = FC // 2
NCH = F // FC
f32, bf16, u32 = jnp.float32, jnp.bfloat16, jnp.uint32


def _gelu(x):
    c = float(np.sqrt(2.0 / np.pi))
    return x * (0.5 * (1.0 + jnp.tanh(c * (x + 0.044715 * (x * x * x)))))


def _lhs_terms(a11, a12, a21, a22):
    return (a11 + a22, a21 + a22, a11, a22, a11 + a12, a21 - a11, a12 - a22)


def _rhs_terms(b11, b12, b21, b22):
    return (b11 + b22, b11, b12 - b22, b21 - b11, b22, b11 + b12, b21 + b22)


def _product(m):
    m1, m4 = m(0), m(3)
    c11 = m1 + m4
    m2 = m(1)
    c21 = m2 + m4
    c22 = m1 - m2
    m3 = m(2)
    c22 = c22 + m3
    m5 = m(4)
    c12 = m3 + m5
    c11 = c11 - m5
    c11 = c11 + m(6)
    c22 = c22 + m(5)
    return c11, c12, c21, c22


def _ds(start, size, align):
    if isinstance(start, int):
        return pl.ds(start, size)
    return pl.ds(pl.multiple_of(start, align), size)


def build(G=16, M1=128, M2=256, M3=512, M4=256, AG=6, qk_st=8, pv_st=8, scopes=False, nobc=False, PR=16, PG=16, qgate=1, c1=1, q_per=1, slow2=True, gu_per=5, d_per=8, ogate=False, gap=32, st=1, t1=3, lnr=1, late=1, MQ=256, c2=False,
          gmode='half', qk_done=0, sm_st=2, sm_done=0, pv_done=0, pv_slow=0, only=None):
    N1, N2, N3, N4 = HS // M1, HS // M2, HS // M3, HS // M4
    assert N2 == NC // 2
    K1 = HD // N1

    import contextlib
    scope = jax.named_scope if scopes else (lambda n: contextlib.nullcontext())

    def kern(x_hbm, wqkv_hbm, wo_hbm, wg_hbm, wu_hbm, wd_hbm, out_hbm,
             x_v, xa, ha, ha_last, oa, acc, q_s, k_s, v_s,
             bq, bkv, bo, bgu, bd, bd_last, rqkv, ro, ro_f, rg, ru, rd,
             xsem, qsem, kvsem, gsem, usem, dsem, osem, wosem):

        def x_copy(i):
            rows = _ds(i * 2 * M1, 2 * M1, 2 * M1)
            return pltpu.make_async_copy(x_hbm.at[rows], x_v.at[rows], xsem.at[i])

        def qkv_copy(i):
            rows = _ds(i * K1, K1, K1)
            return pltpu.make_async_copy(wqkv_hbm.at[:, rows, pl.ds(0, D)], rqkv.at[:, rows, pl.ds(0, D)], qsem.at[i])

        def kv_copy(i):
            rows = _ds(i * K1, K1, K1)
            return pltpu.make_async_copy(
                wqkv_hbm.at[:, rows, pl.ds(D, 2 * D)], rqkv.at[:, rows, pl.ds(D, 2 * D)], kvsem.at[i])

        def g_copy(c):
            return pltpu.make_async_copy(wg_hbm.at[:, _ds(c * FC, FC, FC)], rg.at[c % 2], gsem.at[c % 2])

        def u_copy(c):
            return pltpu.make_async_copy(wu_hbm.at[:, _ds(c * FC, FC, FC)], ru.at[c % 2], usem.at[c % 2])

        def d_copy(c):
            return pltpu.make_async_copy(wd_hbm.at[_ds(c * FC, FC, FC)], rd.at[c % 2], dsem.at[c % 2])

        wo_copy = pltpu.make_async_copy(wo_hbm, ro, wosem.at[0])

        def out_copy(i, half):
            at = (_ds(i * 2 * M4, 2 * M4, 2 * M4), pl.ds(half * HD, HD))
            return pltpu.make_async_copy(x_v.at[at], out_hbm.at[at], osem.at[2 * i + half])

        def get(ref, rows=None):
            at = slice(None) if rows is None else _ds(rows[0] // 2, rows[1] // 2, rows[1] // 2)
            return pltpu.bitcast(ref[at, :], bf16)

        def put(ref, rows, c0, t):
            at = _ds(rows[0] // 2, rows[1] // 2, rows[1] // 2)
            ref[at, _ds(c0 * 128, t.shape[1], 128)] = pltpu.bitcast(t.astype(bf16), u32)

        ha_j = lambda j: ha.at[j] if j < 6 else ha_last
        bd_j = lambda c, j: bd.at[c % 2, j] if j < 6 else bd_last.at[c % 2]

        class Chain:
            def __init__(self, never):
                self.never, self.last = never, None

            def gate(self, t):
                if self.never is None or self.last is None:
                    return t
                last = self.last if self.last.dtype == t.dtype else pltpu.bitcast(self.last, t.dtype)
                if last.shape != t.shape:
                    last = jnp.tile(last, (t.shape[0] // 8, t.shape[1] // 128))
                return jnp.where(self.never, last, t)

            def done(self, t, slow=False):
                if self.never is not None:
                    t = t[:8, :128]
                    self.last = pltpu.roll(t, 1, 1) if slow else t

        def rhs_piece(chain, slow, b11, b12, b21, b22):
            terms = _rhs_terms(chain.gate(b11), b12, b21, chain.gate(b22))
            chain.done(terms[0], slow)
            return terms

        def layernorm(i, chain):
            for g in range(M1 // G):
                halves = []
                for t in range(lnr):
                    n = 2 * G // lnr
                    x = chain.gate(x_v[_ds(i * 2 * M1 + 2 * G * g + n * t, n, G), :].astype(f32))
                    mean = jnp.mean(x, axis=-1, keepdims=True)
                    xc = x - mean
                    var = jnp.mean(xc * xc, axis=-1, keepdims=True)
                    halves.append(xc * lax.rsqrt(var + 1e-5))
                    if lnr > 1:
                        chain.done(xc)
                xn = jnp.concatenate(halves, axis=0)
                terms = _lhs_terms(xn[:G, :HD], xn[:G, HD:], xn[G:, :HD], xn[G:, HD:])
                for j, t in enumerate(terms):
                    put(xa.at[j], (i * M1 + G * g, G), 0, t)
                if lnr == 1:
                    chain.done(terms[0])
                yield

        def prep_qkv(i, n, parts, chain):
            lane = lax.broadcasted_iota(jnp.int32, (PR // 2, 128), 1)
            grp = (lane >> 2) & 7
            for r in range(0, HD // n, PR):
                rows = _ds(i * (HD // n) + r, PR, PR)
                for part in parts:
                    halves = []
                    for half in range(2):
                        a = []
                        for cs in range(NC):
                            cd = (grp - cs) & 7
                            dl = ((lane >> 5) - (grp < cd).astype(jnp.int32)) & 3
                            idx = (lane & 3) * 32 + cd * 4 + dl
                            w = pltpu.bitcast(rqkv[half, rows, pl.ds(part * D + cs * 128, 128)], u32)
                            a.append(jnp.take_along_axis(chain.gate(w), idx, axis=1))
                        a = [a[(-j) % 8] for j in range(8)]
                        for b in (1, 2, 4):
                            sel = (grp & b) != 0
                            a = [jnp.where(sel, a[(j - b) % 8], a[j]) for j in range(8)]
                        a = [a[cd] if cd == 0 else pltpu.roll(a[cd], 128 - 4 * cd, 1) for cd in range(NC)]
                        halves.append(a)
                    if qgate == 0:
                        chain.done(halves[1][-1])
                    for c in range(0, NC // 2, 2):
                        ld = lambda half, cc: pltpu.bitcast(
                            jnp.concatenate(halves[half][cc:cc + 2], axis=1), bf16).astype(f32)
                        terms = _rhs_terms(ld(0, c), ld(0, c + 4), ld(1, c), ld(1, c + 4))
                        for j, t in enumerate(terms):
                            put(bq.at[j] if part == 0 else bkv.at[part - 1, j], (i * (HD // n) + r, PR), c, t)
                    if qgate == 1:
                        chain.done(terms[0])
                    yield

        def prep_wo(i, chain, slow):
            for half in range(2):
                cols = _ds((i + 4 * half) * 128, 128, 128)
                for h in range(H):
                    t = chain.gate(ro[pl.ds(h * DH, DH), cols].astype(f32))
                    ro_f[half, pl.ds(h * (DH + 1), DH), :] = t
                    chain.done(t, slow and h % 4 == 3)
                    yield
            for d in range(DH // 2):
                ld = lambda half, dd: ro_f[half, pl.ds(dd, H, stride=DH + 1), :]
                terms = rhs_piece(chain, slow, ld(0, d), ld(1, d), ld(0, d + DH // 2), ld(1, d + DH // 2))
                for j, t in enumerate(terms):
                    put(bo.at[j], (d * H, H), i, t)
                yield

        def prep_gu(c, i, n, chain, slow, which=((0, rg), (HC, ru))):
            kp = HD // n
            for r in range(0, kp, PG):
                lo, hi = _ds(i * kp + r, PG, PG), _ds(HD + i * kp + r, PG, PG)
                for off, raw in which:
                    ld = lambda rr, o: raw[c % 2, rr, pl.ds(o, HC)].astype(f32)
                    terms = rhs_piece(chain, slow, ld(lo, 0), ld(lo, HC), ld(hi, 0), ld(hi, HC))
                    for j, t in enumerate(terms):
                        put(bgu.at[c % 2, j], (i * kp + r, PG), off // 128, t)
                    yield

        def prep_d(c, i, n, chain, slow):
            kp = HC // n
            for r in range(0, kp, PG):
                lo, hi = _ds(i * kp + r, PG, PG), _ds(HC + i * kp + r, PG, PG)
                for o in range(0, HD, 256):
                    ld = lambda rr, oo: rd[c % 2, rr, pl.ds(oo + o, 256)].astype(f32)
                    terms = rhs_piece(chain, slow, ld(lo, 0), ld(lo, HD), ld(hi, 0), ld(hi, HD))
                    for j, t in enumerate(terms):
                        put(bd_j(c, j), (i * kp + r, PG), o // 128, t)
                    yield

        def run(*jobs):
            jobs = list(jobs)
            while jobs:
                for job in list(jobs):
                    gen, n = job
                    for _ in range(n):
                        if next(gen, "end") == "end":
                            jobs.remove(job)
                            break

        def gate_up(c, rows, before_store=None):
            quads = _product(lambda j: jnp.dot(get(xa.at[j], rows), get(bgu.at[c % 2, j]), preferred_element_type=f32))
            hs = [_gelu(t[:, :HC]) * t[:, HC:] for t in quads]
            if before_store is not None:
                before_store()
            for j, t in enumerate(_lhs_terms(*hs)):
                put(ha_j(j), rows, 0, t)

        log2e = float(np.log2(np.e))
        scale = DH ** -0.5

        def attention8(base, r, chain, outs):
            q = [q_s[c, _ds(base + r, 8, 8), :] for c in range(NC)]
            ls = []
            for w in range(W):
                if gmode == "q" and w % (W // qk_st) == 0:
                    q = [chain.gate(t) for t in q]
                if gmode == "half":
                    q = [chain.gate(t) if c % 2 == w % 2 else t for c, t in enumerate(q)]
                at = pl.ds(base + (HALO + r - DIL * w), 8)
                p = q[0] * k_s[0, at, :]
                if gmode == "acc":
                    p = chain.gate(p)
                for c in range(1, NC):
                    p = p + q[c] * k_s[c, at, :]
                if qk_done == 0:
                    chain.done(p)
                p = p + pltpu.roll(p, 64, 1)
                if qk_done == 1:
                    chain.done(p)
                p = p + pltpu.roll(p, 32, 1)
                if qk_done == 2:
                    chain.done(p)
                if r < DIL * w:
                    pos = base + r + lax.broadcasted_iota(jnp.int32, (8, 128), 0)
                    p = jnp.where(pos >= DIL * w, p, -1e9 * log2e)
                ls.append(p)
                yield
            m = functools.reduce(jnp.maximum, ls)
            ps = []
            for w, l in enumerate(ls):
                if sm_st and w and w % sm_st == 0:
                    m = jnp.where(chain.never, ps[-1], m)
                ps.append(jnp.exp2(l - m))
            inv = 1.0 / functools.reduce(jnp.add, ps)
            if sm_done:
                chain.done(inv if sm_done == 1 else ps[-1])
                ps = [chain.gate(t) for t in ps]
            for n, c in enumerate((0, 1, 4, 5, 2, 3, 6, 7)):
                if gmode == "q" and n and n % (NC // pv_st) == 0:
                    ps = [chain.gate(t) for t in ps]
                if gmode == "half" and n:
                    ps = [chain.gate(t) if w % 2 == n % 2 else t for w, t in enumerate(ps)]
                o = ps[0] * v_s[c, pl.ds(base + (HALO + r), 8), :]
                if gmode == "acc" and n:
                    o = chain.gate(o)
                for w in range(1, W):
                    o = o + ps[w] * v_s[c, pl.ds(base + (HALO + r - DIL * w), 8), :]
                outs[c] = o * inv
                chain.done(outs[c] if pv_done else o, pv_slow and n % pv_slow == pv_slow - 1)
                yield

        def attention(g0, chain):
            base = g0 * (2 * G)
            for g in range(AG):
                parts = []
                for r in range(2 * G * g, 2 * G * (g + 1), 8):
                    parts.append({})
                    yield from attention8(base, r, chain, parts[-1])
                n = G // 8
                quad = lambda p, c: jnp.concatenate(
                    [jnp.concatenate([parts[p * n + t][c], parts[p * n + t][c + 1]], axis=1) for t in range(n)], axis=0)
                for c in range(0, NC // 2, 2):
                    terms = _lhs_terms(quad(0, c), quad(0, c + 4), quad(1, c), quad(1, c + 4))
                    for j, t in enumerate(terms):
                        put(oa.at[j], ((g0 + g) * G, G), c, t)
                    if ogate:
                        chain.done(terms[0])

        x_copy(0).start()
        g_copy(0).start()
        if st == 0:
            u_copy(0).start()
            x_copy(1).start()
            qkv_copy(0).start()
        with scope("s0_x0"):
            x_copy(0).wait()
        if st >= 1:
            u_copy(0).start()
        if st == 1:
            x_copy(1).start()
            qkv_copy(0).start()
        with scope("s1_ln0"):
            run((layernorm(0, Chain(None)), 1))
        if st == 2:
            x_copy(1).start()
            qkv_copy(0).start()
        with scope("s2_gu0"):
            g_copy(0).wait()
            if st == 3:
                x_copy(1).start()
                qkv_copy(0).start()
            run((prep_gu(0, 0, 1, Chain(None), False, ((0, rg),)), 1))
            u_copy(0).wait()
        with scope("s3_prep0"):
            run((prep_gu(0, 0, 1, Chain(None), False, ((HC, ru),)), 1))

        def stage1(i, carry):
            pl.when(i + 2 < N1)(x_copy(jnp.minimum(i + 2, N1 - 1)).start)
            pl.when(i + 1 < N1)(qkv_copy(jnp.minimum(i + 1, N1 - 1)).start)
            kv_copy(i).start()
            nxt = jnp.minimum(i + 1, N1 - 1)
            pl.when(i + 1 < N1)(x_copy(nxt).wait)
            qkv_copy(i).wait()
            gate_up(0, (i * M1, M1))
            ca = Chain(i < 0 if c1 in (1, 3) else None)
            cb = ca if c1 == 3 else Chain(i < 0 if c1 in (1, 2) else None)
            run(*([(layernorm(nxt, ca), 1)] if t1 & 1 else []), *([(prep_qkv(i, N1, (0,), cb), q_per)] if t1 & 2 else []))
            return carry

        with scope("s4_stage1"):
            if only in (None, 1): lax.fori_loop(0, N1, stage1, 0)

        def project(i, m, terms, dst, off, mult=None):
            rows = (i * m, m)
            quads = _product(lambda j: jnp.dot(get(xa.at[j], rows), get(terms.at[j]), preferred_element_type=f32))
            for k, t in enumerate(quads):
                if mult is not None:
                    t = t * mult
                for g in range(m // G):
                    at = _ds(i * 2 * m + (off + 2 * G * g + G * (k // 2)), G, G)
                    for c in range(NC // 2):
                        dst[c + 4 * (k % 2), at, :] = t[G * g:G * (g + 1), c * 128:(c + 1) * 128]

        for cp in (wo_copy, d_copy(0), g_copy(1), u_copy(1)):
            cp.start()
        with scope("s5_wait"):
            for i in range(N1):
                kv_copy(i).wait()

        def stage2q(i, carry):
            project(i, MQ, bq, q_s, 0, scale * log2e)
            run((prep_qkv(i, HS // MQ, (1, 2), Chain(i < 0 if c2 else None)), 1))
            return carry

        with scope("s6_stage2q"):
            if only in (None, 2): lax.fori_loop(0, HS // MQ, stage2q, 0)
        for cp in (d_copy(1), g_copy(2), u_copy(2)):
            cp.start()
        for cp in (wo_copy, d_copy(0), g_copy(1), u_copy(1)):
            cp.wait()

        def stage2kv(i, carry):
            project(i, M2, bkv.at[0], k_s, HALO)
            project(i, M2, bkv.at[1], v_s, HALO)
            chain = Chain(i < 0)
            run((prep_wo(i, chain, slow2), 1000), (prep_d(0, i, N2, chain, slow2), 1000), (prep_gu(1, i, N2, chain, slow2), 1000))
            return carry

        with scope("s6_stage2kv"):
            if only in (None, 2): lax.fori_loop(0, N2, stage2kv, 0)
        for c in range(NC):
            k_s[c, pl.ds(0, HALO), :] = jnp.zeros((HALO, 128), f32)
            v_s[c, pl.ds(0, HALO), :] = jnp.broadcast_to(v_s[c, pl.ds(HALO, 1), :], (HALO, 128))

        def stage3(t, carry):
            c, i = t // N3, t % N3

            @pl.when(i == 0)
            def _():
                pl.when(c + 2 < NCH)(d_copy(jnp.minimum(c + 2, NCH - 1)).start)
                pl.when(c + 3 < NCH)(g_copy(jnp.minimum(c + 3, NCH - 1)).start)
                pl.when(c + 3 < NCH)(u_copy(jnp.minimum(c + 3, NCH - 1)).start)
                d_copy(c + 1).wait()
                pl.when(c + 2 < NCH)(g_copy(jnp.minimum(c + 2, NCH - 1)).wait)
                pl.when(c + 2 < NCH)(u_copy(jnp.minimum(c + 2, NCH - 1)).wait)

            rows = _ds(i * M3, M3, M3)
            def down(j):
                acc[j, rows, :] = jnp.where(c > 0, acc[j, rows, :], 0.0) + jnp.dot(
                    get(ha_j(j), (i * M3, M3)), get(bd_j(c, j)), preferred_element_type=f32)

            for j in range(7 - late):
                down(j)
            chain = Chain(t < 0)
            att = attention(jnp.minimum(t * AG, HS // G - AG), chain)
            for _ in prep_gu(c + 2, i, N3, chain, False):
                for _ in range(gu_per):
                    next(att)
            gate_up(c + 1, (i * M3, M3), (lambda: down(6)) if late else None)
            for _ in range(gap):
                next(att)
            run((prep_d(c + 1, i, N3, chain, False), 1), (att, d_per))
            return carry

        with scope("s7_stage3"):
            if only in (None, 3): lax.fori_loop(0, (NCH - 1) * N3, stage3, 0)

        def stage4(i, carry):
            m = lambda j: (acc[j, _ds(i * M4, M4, M4), :]
                           + jnp.dot(get(ha_j(j), (i * M4, M4)), get(bd_j(NCH - 1, j)), preferred_element_type=f32)
                           + jnp.dot(get(oa.at[j], (i * M4, M4)), get(bo.at[j]), preferred_element_type=f32))

            def finish(t, bottom, half):
                for g in range(M4 // G):
                    at = (_ds(i * 2 * M4 + (2 * G * g + G * bottom), G, G), pl.ds(half * HD, HD))
                    x_v[at] = (x_v[at].astype(f32) + t[G * g:G * (g + 1)]).astype(bf16)

            m1, m4, m5 = m(0), m(3), m(4)
            finish(m1 + m4 - m5 + m(6), 0, 0)
            m2 = m(1)
            finish(m2 + m4, 1, 0)
            out_copy(i, 0).start()
            m3 = m(2)
            finish(m3 + m5, 0, 1)
            finish(m1 - m2 + m3 + m(5), 1, 1)
            out_copy(i, 1).start()
            return carry

        with scope("s8_stage4"):
            if only in (None, 4): lax.fori_loop(0, N4, stage4, 0)
        with scope("s9_tail"):
            for i in range(N4):
                out_copy(i, 0).wait()
                out_copy(i, 1).wait()

    def f(A_x, A_wqkv, A_wo, B_x, B_w_gate, B_w_up, B_w_down):
        anyspec = pl.BlockSpec(memory_space=pl.ANY)
        dma = pltpu.SemaphoreType.DMA
        vmem = pltpu.VMEM
        out = pl.pallas_call(
            kern,
            in_specs=[anyspec] * 6,
            out_specs=anyspec,
            out_shape=jax.ShapeDtypeStruct((S, D), bf16),
            scratch_shapes=[
                vmem((S, D), bf16),
                vmem((7, HS // 2, HD), u32), vmem((6, HS // 2, HC), u32), vmem((HS // 2, HC), u32),
                vmem((7, HS // 2, HD), u32), vmem((7, HS, HD), f32),
                vmem((NC, S, 128), f32), vmem((NC, S + HALO, 128), f32), vmem((NC, S + HALO, 128), f32),
                vmem((7, HD // 2, HD), u32), vmem((2, 7, HD // 2, HD), u32), vmem((7, HD // 2, HD), u32),
                vmem((2, 7, HD // 2, FC), u32), vmem((2, 6, HC // 2, HD), u32), vmem((2, HC // 2, HD), u32),
                vmem((2, HD, 3 * D), bf16), vmem((D, D), bf16), vmem((2, H * (DH + 1), 128), f32),
                vmem((2, D, FC), bf16), vmem((2, D, FC), bf16), vmem((2, FC, D), bf16),
                dma((N1,)), dma((N1,)), dma((N1,)), dma((2,)), dma((2,)), dma((2,)), dma((2 * N4,)), dma((1,)),
            ],
            compiler_params=pltpu.CompilerParams(vmem_limit_bytes=124 * 1024 * 1024, disable_bounds_checks=nobc),
        )(A_x.reshape(S, D), A_wqkv.reshape(2, HD, 3 * D), A_wo, B_w_gate, B_w_up, B_w_down)
        return out.reshape(1, S, D)
    return f


@jax.jit
def pallas_parallel_sum__sliding_local_dilated__glu_gated_geglu__prompt_kernel(
    A_x, A_wqkv, A_wo, B_x, B_w_gate, B_w_up, B_w_down):
    return build()(A_x, A_wqkv, A_wo, B_x, B_w_gate, B_w_up, B_w_down)
```

```python
import functools

import jax
import jax.numpy as jnp
import numpy as np
from jax import lax
from jax.experimental import pallas as pl
from jax.experimental.pallas import tpu as pltpu

S, D, F = 2048, 1024, 3584
H, DH, W, DIL = 32, 32, 8, 2
EPS, MASKED = 1e-5, -1e9

LANES = 128
NC = D // LANES
HS, HD = S // 2, D // 2
G = 16
HALO = 16
FC = 512
HC = FC // 2
NCH = F // FC
M1, M2, M3, M4 = 128, 256, 512, 256
N1, N2, N3, N4 = HS // M1, HS // M2, HS // M3, HS // M4
AG = -(-(HS // G) // ((NCH - 1) * N3))
LOG2E = float(np.log2(np.e))
Q_SCALE = DH ** -0.5 * LOG2E

f32, bf16, u32 = jnp.float32, jnp.bfloat16, jnp.uint32


def _gelu(x):
    c = float(np.sqrt(2.0 / np.pi))
    return x * (0.5 * (1.0 + jnp.tanh(c * (x + 0.044715 * (x * x * x)))))


def _dot(a, b):
    return jnp.dot(a, b, preferred_element_type=f32)


def _lhs_terms(a11, a12, a21, a22):
    return (a11 + a22, a21 + a22, a11, a22, a11 + a12, a21 - a11, a12 - a22)


def _rhs_terms(b11, b12, b21, b22):
    return (b11 + b22, b11, b12 - b22, b21 - b11, b22, b11 + b12, b21 + b22)


def _quadrants(m):
    m1, m4 = m(0), m(3)
    c11 = m1 + m4
    m2 = m(1)
    c21 = m2 + m4
    c22 = m1 - m2
    m3 = m(2)
    c22 = c22 + m3
    m5 = m(4)
    c12 = m3 + m5
    c11 = c11 - m5
    c11 = c11 + m(6)
    c22 = c22 + m(5)
    return c11, c12, c21, c22


def _ds(start, size, align):
    if isinstance(start, int):
        return pl.ds(start, size)
    return pl.ds(pl.multiple_of(start, align), size)


def _get(ref, start=None, size=None):
    rows = slice(None) if start is None else _ds(start // 2, size // 2, size // 2)
    return pltpu.bitcast(ref[rows, :], bf16)


def _put(ref, start, tile, t):
    words = t.shape[0] // 2
    ref[_ds(start // 2, words, words), _ds(tile * LANES, t.shape[1], LANES)] = pltpu.bitcast(
        t.astype(bf16), u32)


class _Chain:
    def __init__(self, never):
        self.never, self.last = never, None

    def gate(self, t):
        if self.never is None or self.last is None:
            return t
        last = self.last if self.last.dtype == t.dtype else pltpu.bitcast(self.last, t.dtype)
        if last.shape != t.shape:
            last = jnp.tile(last, (t.shape[0] // 8, t.shape[1] // LANES))
        return jnp.where(self.never, last, t)

    def done(self, t, slow=False):
        if self.never is not None:
            t = t[:8, :LANES]
            self.last = pltpu.roll(t, 1, 1) if slow else t


def _run(*jobs):
    jobs = list(jobs)
    while jobs:
        for job in list(jobs):
            gen, n = job
            for _ in range(n):
                if next(gen, "end") == "end":
                    jobs.remove(job)
                    break


def _kernel(x_hbm, wqkv_hbm, wo_hbm, wg_hbm, wu_hbm, wd_hbm, out_hbm,
            x_v, xa_even, xa_odd, ha, ha_last, oa, acc, q_s, k_s, v_s,
            bq, bkv, bo, bgu, bd, bd_last, rqkv, ro, ro_f, rg, ru, rd,
            xsem, qsem, kvsem, gsem, usem, dsem, osem, wosem):
    xa = (xa_even, xa_odd)
    ha_j = lambda j: ha.at[j] if j < 6 else ha_last
    bd_j = lambda c, j: bd.at[c % 2, j] if j < 6 else bd_last.at[c % 2]

    def get_x(j, i, m):
        n = m // (2 * M1)
        return jnp.concatenate(
            [_get(xa[odd].at[j], (i * n + p) * M1, M1) for p in range(n) for odd in range(2)], axis=0)

    def x_copy(i):
        rows = _ds(i * 2 * M1, 2 * M1, 2 * M1)
        return pltpu.make_async_copy(x_hbm.at[rows], x_v.at[rows], xsem.at[i])

    def q_copy(p):
        n = HD // (N1 // 2)
        at = (slice(None), _ds(p * n, n, n), pl.ds(0, D))
        return pltpu.make_async_copy(wqkv_hbm.at[at], rqkv.at[at], qsem.at[p])

    def kv_copy(i):
        n = HD // N1
        at = (slice(None), _ds(i * n, n, n), pl.ds(D, 2 * D))
        return pltpu.make_async_copy(wqkv_hbm.at[at], rqkv.at[at], kvsem.at[i])

    def g_copy(c):
        return pltpu.make_async_copy(wg_hbm.at[:, _ds(c * FC, FC, FC)], rg.at[c % 2], gsem.at[c % 2])

    def u_copy(c):
        return pltpu.make_async_copy(wu_hbm.at[:, _ds(c * FC, FC, FC)], ru.at[c % 2], usem.at[c % 2])

    def d_copy(c):
        return pltpu.make_async_copy(wd_hbm.at[_ds(c * FC, FC, FC)], rd.at[c % 2], dsem.at[c % 2])

    wo_copy = pltpu.make_async_copy(wo_hbm, ro, wosem.at[0])

    def out_copy(i, half):
        at = (_ds(i * 2 * M4, 2 * M4, 2 * M4), pl.ds(half * HD, HD))
        return pltpu.make_async_copy(x_v.at[at], out_hbm.at[at], osem.at[2 * i + half])

    def layernorm(p, odd, chain):
        for g in range(M1 // G):
            xn = []
            for bottom in range(2):
                row = (2 * p + odd) * 2 * M1 + 2 * G * g + G * bottom
                x = chain.gate(x_v[_ds(row, G, G), :].astype(f32))
                xc = x - jnp.mean(x, axis=-1, keepdims=True)
                var = jnp.mean(xc * xc, axis=-1, keepdims=True)
                xn.append(xc * lax.rsqrt(var + EPS))
                chain.done(xc)
            terms = _lhs_terms(xn[0][:, :HD], xn[0][:, HD:], xn[1][:, :HD], xn[1][:, HD:])
            for j, t in enumerate(terms):
                _put(xa[odd].at[j], p * M1 + G * g, 0, t)
            yield

    def prep_qkv(i, n, parts, chain):
        lane = lax.broadcasted_iota(jnp.int32, (G // 2, LANES), 1)
        grp = (lane >> 2) & 7
        for r in range(0, HD // n, G):
            row = i * (HD // n) + r
            for part in parts:
                halves = []
                for half in range(2):
                    a = []
                    for src in range(NC):
                        dst = (grp - src) & 7
                        quarter = ((lane >> 5) - (grp < dst).astype(jnp.int32)) & 3
                        idx = (lane & 3) * DH + dst * 4 + quarter
                        w = rqkv[half, _ds(row, G, G), pl.ds(part * D + src * LANES, LANES)]
                        a.append(jnp.take_along_axis(chain.gate(pltpu.bitcast(w, u32)), idx, axis=1))
                    a = [a[-j % NC] for j in range(NC)]
                    for b in (1, 2, 4):
                        sel = (grp & b) != 0
                        a = [jnp.where(sel, a[(j - b) % NC], a[j]) for j in range(NC)]
                    halves.append(
                        [t if dst == 0 else pltpu.roll(t, LANES - 4 * dst, 1) for dst, t in enumerate(a)])
                for c in range(0, NC // 2, 2):
                    ld = lambda half, c0: pltpu.bitcast(
                        jnp.concatenate(halves[half][c0:c0 + 2], axis=1), bf16).astype(f32)
                    terms = _rhs_terms(ld(0, c), ld(0, c + NC // 2), ld(1, c), ld(1, c + NC // 2))
                    for j, t in enumerate(terms):
                        _put(bq.at[j] if part == 0 else bkv.at[part - 1, j], row, c, t)
                chain.done(terms[0])
                yield

    def rhs_piece(chain, slow, b11, b12, b21, b22):
        terms = _rhs_terms(chain.gate(b11), b12, b21, chain.gate(b22))
        chain.done(terms[0], slow)
        return enumerate(terms)

    def prep_wo(i, chain):
        pitch = DH + 1
        for half in range(2):
            cols = _ds((i + half * NC // 2) * LANES, LANES, LANES)
            for h in range(H):
                t = chain.gate(ro[pl.ds(h * DH, DH), cols].astype(f32))
                ro_f[half, pl.ds(h * pitch, DH), :] = t
                chain.done(t, h % 4 == 3)
                yield
        for d in range(DH // 2):
            ld = lambda half, d0: ro_f[half, pl.ds(d0, H, stride=pitch), :]
            for j, t in rhs_piece(chain, True, ld(0, d), ld(1, d), ld(0, d + DH // 2), ld(1, d + DH // 2)):
                _put(bo.at[j], d * H, i, t)
            yield

    def prep_gu(c, i, n, chain, slow=False, which=(0, 1)):
        for r in range(0, HD // n, G):
            row = i * (HD // n) + r
            for side in which:
                ld = lambda r0, c0: (rg, ru)[side][c % 2, _ds(r0, G, G), pl.ds(c0, HC)].astype(f32)
                for j, t in rhs_piece(chain, slow, ld(row, 0), ld(row, HC), ld(HD + row, 0), ld(HD + row, HC)):
                    _put(bgu.at[c % 2, j], row, side * HC // LANES, t)
                yield

    def prep_d(c, i, n, chain, slow=False):
        for r in range(0, HC // n, G):
            row = i * (HC // n) + r
            for col in range(0, HD, 2 * LANES):
                ld = lambda r0, c0: rd[c % 2, _ds(r0, G, G), pl.ds(c0 + col, 2 * LANES)].astype(f32)
                for j, t in rhs_piece(chain, slow, ld(row, 0), ld(row, HD), ld(HC + row, 0), ld(HC + row, HD)):
                    _put(bd_j(c, j), row, col // LANES, t)
                yield

    def attention8(base, r, chain, out):
        q = [q_s[c, _ds(base + r, 8, 8), :] for c in range(NC)]
        window = [pl.ds(base + (HALO + r - DIL * w), 8) for w in range(W)]
        logits = []
        for w in range(W):
            q = [chain.gate(t) if c % 2 == w % 2 else t for c, t in enumerate(q)]
            t = q[0] * k_s[0, window[w], :]
            for c in range(1, NC):
                t = t + q[c] * k_s[c, window[w], :]
            chain.done(t)
            t = t + pltpu.roll(t, 2 * H, 1)
            t = t + pltpu.roll(t, H, 1)
            if r < DIL * w:
                pos = base + r + lax.broadcasted_iota(jnp.int32, (8, LANES), 0)
                t = jnp.where(pos >= DIL * w, t, MASKED * LOG2E)
            logits.append(t)
            yield
        top = functools.reduce(jnp.maximum, logits)
        e = []
        for w, t in enumerate(logits):
            if w and w % 2 == 0:
                top = jnp.where(chain.never, e[-1], top)
            e.append(jnp.exp2(t - top))
        inv = 1.0 / functools.reduce(jnp.add, e)
        for n, c in enumerate((0, 1, 4, 5, 2, 3, 6, 7)):
            if n:
                e = [chain.gate(t) if w % 2 == n % 2 else t for w, t in enumerate(e)]
            o = e[0] * v_s[c, window[0], :]
            for w in range(1, W):
                o = o + e[w] * v_s[c, window[w], :]
            out[c] = o * inv
            chain.done(o)
            yield

    def attention(g0, chain):
        base = g0 * (2 * G)
        for g in range(AG):
            parts = []
            for r in range(2 * G * g, 2 * G * (g + 1), 8):
                parts.append({})
                yield from attention8(base, r, chain, parts[-1])
            block = lambda bottom, c: jnp.concatenate(
                [jnp.concatenate([parts[2 * bottom + t][c], parts[2 * bottom + t][c + 1]], axis=1)
                 for t in range(2)], axis=0)
            for c in range(0, NC // 2, 2):
                terms = _lhs_terms(block(0, c), block(0, c + NC // 2), block(1, c), block(1, c + NC // 2))
                for j, t in enumerate(terms):
                    _put(oa.at[j], (g0 + g) * G, c, t)

    def gate_up(c, row, lhs, before_store=None):
        quads = _quadrants(lambda j: _dot(lhs(j), _get(bgu.at[c % 2, j])))
        h = [_gelu(t[:, :HC]) * t[:, HC:] for t in quads]
        if before_store is not None:
            before_store()
        for j, t in enumerate(_lhs_terms(*h)):
            _put(ha_j(j), row, 0, t)

    def project(i, terms, dst, first_row, scale=None):
        quads = _quadrants(lambda j: _dot(get_x(j, i, M2), _get(terms.at[j])))
        for k, t in enumerate(quads):
            if scale is not None:
                t = t * scale
            for g in range(M2 // G):
                rows = _ds(i * 2 * M2 + (first_row + 2 * G * g + G * (k // 2)), G, G)
                for c in range(NC // 2):
                    dst[c + (k % 2) * NC // 2, rows, :] = t[G * g:G * (g + 1), c * LANES:(c + 1) * LANES]

    for cp in (x_copy(0), g_copy(0), u_copy(0), x_copy(1)):
        cp.start()
    x_copy(0).wait()
    _run((layernorm(0, 0, _Chain(None)), 1))
    g_copy(0).wait()
    _run((prep_gu(0, 0, 1, _Chain(None), which=(0,)), 1))
    u_copy(0).wait()
    _run((prep_gu(0, 0, 1, _Chain(None), which=(1,)), 1))

    def stage1(p, carry):
        for odd in range(2):
            i = 2 * p + odd
            pl.when(i + 2 < N1)(x_copy(jnp.minimum(i + 2, N1 - 1)).start)
            if not odd:
                q_copy(p).start()
            kv_copy(i).start()
            pl.when(i + 1 < N1)(x_copy(jnp.minimum(i + 1, N1 - 1)).wait)
            if odd:
                q_copy(p).wait()
            gate_up(0, i * M1, lambda j: _get(xa[odd].at[j], p * M1, M1))
            jobs = [(layernorm(jnp.minimum(p + odd, N1 // 2 - 1), 1 - odd, _Chain(p < 0)), 1)]
            if odd:
                jobs.append((prep_qkv(p, N1 // 2, (0,), _Chain(p < 0)), 1))
            _run(*jobs)
        return carry

    lax.fori_loop(0, N1 // 2, stage1, 0)

    for cp in (wo_copy, d_copy(0), g_copy(1), u_copy(1)):
        cp.start()
    for i in range(N1):
        kv_copy(i).wait()

    def stage2_q(i, carry):
        project(i, bq, q_s, 0, Q_SCALE)
        _run((prep_qkv(i, N2, (1, 2), _Chain(None)), 1))
        return carry

    lax.fori_loop(0, N2, stage2_q, 0)
    for cp in (d_copy(1), g_copy(2), u_copy(2)):
        cp.start()
    for cp in (wo_copy, d_copy(0), g_copy(1), u_copy(1)):
        cp.wait()

    def stage2_kv(i, carry):
        project(i, bkv.at[0], k_s, HALO)
        project(i, bkv.at[1], v_s, HALO)
        chain = _Chain(i < 0)
        _run((prep_wo(i, chain), 1))
        _run((prep_d(0, i, N2, chain, slow=True), 1))
        _run((prep_gu(1, i, N2, chain, slow=True), 1))
        return carry

    lax.fori_loop(0, N2, stage2_kv, 0)
    for c in range(NC):
        k_s[c, pl.ds(0, HALO), :] = jnp.zeros((HALO, LANES), f32)
        v_s[c, pl.ds(0, HALO), :] = jnp.broadcast_to(v_s[c, pl.ds(HALO, 1), :], (HALO, LANES))

    def stage3(t, carry):
        c, i = t // N3, t % N3

        @pl.when(i == 0)
        def _():
            pl.when(c + 2 < NCH)(d_copy(jnp.minimum(c + 2, NCH - 1)).start)
            pl.when(c + 3 < NCH)(g_copy(jnp.minimum(c + 3, NCH - 1)).start)
            pl.when(c + 3 < NCH)(u_copy(jnp.minimum(c + 3, NCH - 1)).start)
            d_copy(c + 1).wait()
            pl.when(c + 2 < NCH)(g_copy(jnp.minimum(c + 2, NCH - 1)).wait)
            pl.when(c + 2 < NCH)(u_copy(jnp.minimum(c + 2, NCH - 1)).wait)

        def down(j):
            rows = _ds(i * M3, M3, M3)
            acc[j, rows, :] = jnp.where(c > 0, acc[j, rows, :], 0.0) + _dot(
                _get(ha_j(j), i * M3, M3), _get(bd_j(c, j)))

        for j in range(6):
            down(j)
        chain = _Chain(t < 0)
        att = attention(jnp.minimum(t * AG, HS // G - AG), chain)
        for _ in prep_gu(c + 2, i, N3, chain):
            for _ in range(5):
                next(att)
        gate_up(c + 1, i * M3, lambda j: get_x(j, i, M3), lambda: down(6))
        for _ in range(32):
            next(att)
        _run((prep_d(c + 1, i, N3, chain), 1), (att, 8))
        return carry

    lax.fori_loop(0, (NCH - 1) * N3, stage3, 0)

    def stage4(i, carry):
        def m(j):
            return (acc[j, _ds(i * M4, M4, M4), :]
                    + _dot(_get(ha_j(j), i * M4, M4), _get(bd_j(NCH - 1, j)))
                    + _dot(_get(oa.at[j], i * M4, M4), _get(bo.at[j])))

        def finish(t, bottom, half):
            for g in range(M4 // G):
                at = (_ds(i * 2 * M4 + (2 * G * g + G * bottom), G, G), pl.ds(half * HD, HD))
                x_v[at] = (x_v[at].astype(f32) + t[G * g:G * (g + 1)]).astype(bf16)

        m1, m4, m5 = m(0), m(3), m(4)
        finish(m1 + m4 - m5 + m(6), 0, 0)
        m2 = m(1)
        finish(m2 + m4, 1, 0)
        out_copy(i, 0).start()
        m3 = m(2)
        finish(m3 + m5, 0, 1)
        finish(m1 - m2 + m3 + m(5), 1, 1)
        out_copy(i, 1).start()
        return carry

    lax.fori_loop(0, N4, stage4, 0)
    for i in range(N4):
        out_copy(i, 0).wait()
        out_copy(i, 1).wait()


@jax.jit
def pallas_parallel_sum__sliding_local_dilated__glu_gated_geglu__prompt_kernel(
    A_x: jax.Array,
    A_wqkv: jax.Array,
    A_wo: jax.Array,
    B_x: jax.Array,
    B_w_gate: jax.Array,
    B_w_up: jax.Array,
    B_w_down: jax.Array,
):
    del B_x
    vmem, dma = pltpu.VMEM, pltpu.SemaphoreType.DMA
    in_hbm = pl.BlockSpec(memory_space=pl.ANY)
    out = pl.pallas_call(
        _kernel,
        in_specs=[in_hbm] * 6,
        out_specs=in_hbm,
        out_shape=jax.ShapeDtypeStruct((S, D), bf16),
        scratch_shapes=[
            vmem((S, D), bf16),
            vmem((7, HS // 4, HD), u32), vmem((7, HS // 4, HD), u32),
            vmem((6, HS // 2, HC), u32), vmem((HS // 2, HC), u32),
            vmem((7, HS // 2, HD), u32), vmem((7, HS, HD), f32),
            vmem((NC, S, LANES), f32),
            vmem((NC, HALO + S, LANES), f32), vmem((NC, HALO + S, LANES), f32),
            vmem((7, HD // 2, HD), u32), vmem((2, 7, HD // 2, HD), u32),
            vmem((7, HD // 2, HD), u32), vmem((2, 7, HD // 2, FC), u32),
            vmem((2, 6, HC // 2, HD), u32), vmem((2, HC // 2, HD), u32),
            vmem((2, HD, 3 * D), bf16), vmem((D, D), bf16),
            vmem((2, (H + 1) * (DH + 1) - 1, LANES), f32),
            vmem((2, D, FC), bf16), vmem((2, D, FC), bf16), vmem((2, FC, D), bf16),
            dma((N1,)), dma((N1 // 2,)), dma((N1,)), dma((2,)), dma((2,)), dma((2,)),
            dma((2 * N4,)), dma((1,)),
        ],
        compiler_params=pltpu.CompilerParams(
            vmem_limit_bytes=124 * 1024 * 1024, disable_bounds_checks=True),
    )(A_x.reshape(S, D), A_wqkv.reshape(2, HD, 3 * D), A_wo, B_w_gate, B_w_up, B_w_down)
    return out.reshape(1, S, D)
```
